```python
import jax
import jax.numpy as jnp

def _softmax(x, axis=-1):
    return jax.nn.softmax(x, axis=axis)
def _gelu(x):
    return jax.nn.gelu(x, approximate=True)
def _silu(x):
    return jax.nn.silu(x)
def _sigmoid(x):
    return jax.nn.sigmoid(x)
def _layernorm(x, axis=-1, eps=1e-5):
    m = jnp.mean(x, axis=axis, keepdims=True)
    v = jnp.var(x, axis=axis, keepdims=True)
    return (x - m) / jnp.sqrt(v + eps)
def _scatter_add(tgt, idx, src, axis=0):
    return tgt.at[idx].add(src)
def _segment_sum(src, seg, n):
    return jax.ops.segment_sum(src, seg, n)
class _Rng:
    def __init__(self, key):
        self._k = key
    def _next(self):
        self._k, sub = jax.random.split(self._k)
        return sub
    def normal(self, shape):
        return jax.random.normal(self._next(), shape, dtype=jnp.bfloat16)
    def randint(self, lo, hi, shape):
        return jax.random.randint(self._next(), shape, lo, hi, dtype=jnp.int32)
    def uniform(self, shape, lo=0.0, hi=1.0):
        return jax.random.uniform(self._next(), shape, jnp.bfloat16, lo, hi)
    def permutation(self, n):
        return jax.random.permutation(self._next(), n)


kernel_name = 'gated_mix__linear_attn_block__moe_arch_mod__prompt'

def setup_inputs():
    _rng = _Rng(jax.random.key(int.from_bytes(__import__("os").urandom(4), "little")))
    _w = (lambda a: (lambda t: t.astype(jnp.bfloat16) if jnp.issubdtype(t.dtype, jnp.floating) else t)(jnp.asarray(a)))
    def _A_setup():
        B, S, D = 1, 2048, 1024
        return {
            "x": _w((lambda *s: _rng.normal(s) * 0.05)(B, S, D)),
            "wqkv": _w((lambda *s: _rng.normal(s) * 0.05)(D, 3 * D)),
            "wo": _w((lambda *s: _rng.normal(s) * 0.05)(D, D)),
        }
    _A_in = _A_setup()

    def _B_setup():
        B, S, D, F, C = 1, 2048, 1024, 3584, 1
        return {
            "x": _w((lambda *s: _rng.normal(s) * 0.05)(B, S, D)),
            "w_r": _w((lambda *s: _rng.normal(s) * 0.05)(D)),
            "w_gate": _w((lambda *s: _rng.normal(s) * 0.05)(D, F)),
            "w_up": _w((lambda *s: _rng.normal(s) * 0.05)(D, F)),
            "w_down": _w((lambda *s: _rng.normal(s) * 0.05)(F, D)),
        }
    _B_in = _B_setup()

    return {
        "A_x": _A_in["x"],
        "A_wqkv": _A_in["wqkv"],
        "A_wo": _A_in["wo"],
        "B_x": _B_in["x"],
        "B_w_r": _B_in["w_r"],
        "B_w_gate": _B_in["w_gate"],
        "B_w_up": _B_in["w_up"],
        "B_w_down": _B_in["w_down"],
        "gate_w": _w((lambda *s: _rng.normal(s) * 0.05)(1024)),
    }

def reference(A_x, A_wqkv, A_wo, B_x, B_w_r, B_w_gate, B_w_up, B_w_down, gate_w):
    def _A_ref(x, wqkv, wo):
        B, S, D = x.shape
        H = 32; Dh = D // H
        qkv = (lambda x, *d: x.transpose(*d))((x @ wqkv).reshape(B, S, 3, H, Dh), 2, 0, 3, 1, 4)
        q, k, v = qkv[0], qkv[1], qkv[2]
        phi = lambda t: jnp.where(t > 0, t + 1, jnp.exp(t)) + 1e-6
        pq, pk = phi(q), phi(k)
        kv = jnp.einsum("bhsd,bhse->bhde", pk, v)
        z = jnp.einsum("bhsd->bhd", pk)
        num = jnp.einsum("bhqd,bhde->bhqe", pq, kv)
        den = jnp.einsum("bhqd,bhd->bhq", pq, z)[..., None] + 1e-6
        o = num / den
        return (lambda x, *d: x.transpose(*d))(o, 0, 2, 1, 3).reshape(B, S, D) @ wo

    def _B_ref(x, w_r, w_gate, w_up, w_down):
        B, S, D = x.shape
        C = 1
        r = x @ w_r
        idx = jnp.argsort(-r, axis=-1)[:, :C]
        idx_e = jnp.repeat(idx.reshape(B, C, 1), D, axis=2)
        x_sel = jnp.take_along_axis(x, idx_e, axis=1)
        g = _silu(x_sel @ w_gate)
        u = x_sel @ w_up
        y = (g * u) @ w_down
        r_sel = _sigmoid(jnp.take_along_axis(r, idx, axis=1))
        y = y * r_sel.reshape(B, C, 1)
        b_off = (jnp.arange(B) * S).reshape(B, 1)
        flat_idx = (idx + b_off).reshape(B * C)
        zero = (x * 0.0).reshape(B * S, D)
        upd = _scatter_add(zero, flat_idx, y.reshape(B * C, D), axis=0)
        return x + upd.reshape(B, S, D)

    x = A_x
    g = _sigmoid((x * gate_w).sum(-1, keepdims=True))
    a = _A_ref(x, A_wqkv, A_wo)
    b = _B_ref(x, B_w_r, B_w_gate, B_w_up, B_w_down)
    return g * a + (1 - g) * b
```

```python
import jax
import jax.numpy as jnp
from jax import lax
import jax.experimental.pallas as pl
import jax.experimental.pallas.tpu as pltpu

S, D, F, H = 2048, 1024, 3584, 32
DH = D // H
TQ = 512
RK = 256
TO = 512
NQ, NK, NO = S // TQ, D // RK, S // TO
FC = F // NO
F32, BF16 = jnp.float32, jnp.bfloat16


def _phi(t):
    return jnp.where(t > 0, t + 1.0, jnp.exp(t)) + 1e-6


def _sigmoid(t):
    return 1.0 / (1.0 + jnp.exp(-t))


def _rbf(t):
    return t.astype(BF16).astype(F32)


def _rowdot(a, w):
    acc = a[:, 0:128].astype(F32) * w[:, 0:128]
    for j in range(1, D // 128):
        acc = acc + a[:, j * 128:(j + 1) * 128].astype(F32) * w[:, j * 128:(j + 1) * 128]
    return jnp.sum(acc, axis=1, keepdims=True)


def _to_col(row):
    return jnp.broadcast_to(row, (128, row.shape[1])).T


def _kernel(x_hbm, wqkv_hbm, wo_hbm, bx_hbm, wr_ref, wg_hbm, wu_hbm, wd_hbm, gw_ref,
            o_hbm,
            x_v, bx_v, wq_v, wk_v, wv_v, wo_v, wg_v, wu_v, wd_v,
            pq_v, wkt_v, m_v, z_v, g_v, xcol_v, o_v, asel_v,
            s_x, s_bx, s_wq, s_wk, s_wv, s_wo, s_wg, s_wu, s_wd, s_o):

    def rows(i, n):
        return pl.ds(pl.multiple_of(i * n, n), n)

    def cp_x(t):
        return pltpu.make_async_copy(x_hbm.at[rows(t, TQ)], x_v.at[rows(t, TQ)], s_x.at[t])

    def cp_bx(t):
        return pltpu.make_async_copy(bx_hbm.at[rows(t, TQ)], bx_v.at[rows(t, TQ)], s_bx.at[t])

    def cp_wk(t):
        n = D // NQ
        return pltpu.make_async_copy(wqkv_hbm.at[:, pl.ds(pl.multiple_of(D + t * n, n), n)],
                                     wk_v.at[t], s_wk.at[t])

    def cp_wg(c):
        return pltpu.make_async_copy(wg_hbm.at[:, rows(c, FC)], wg_v.at[c], s_wg.at[c])

    def cp_wu(c):
        return pltpu.make_async_copy(wu_hbm.at[:, rows(c, FC)], wu_v.at[c], s_wu.at[c])

    def cp_wd(c):
        return pltpu.make_async_copy(wd_hbm.at[rows(c, FC)], wd_v.at[c], s_wd.at[c])

    def cp_o(t, slot):
        return pltpu.make_async_copy(o_v.at[rows(t, TO)], o_hbm.at[rows(t, TO)], s_o.at[slot])

    cp_wq = pltpu.make_async_copy(wqkv_hbm.at[:, 0:D], wq_v, s_wq.at[0])
    cp_wv = pltpu.make_async_copy(wqkv_hbm.at[:, 2 * D:3 * D], wv_v, s_wv.at[0])
    cp_wo = pltpu.make_async_copy(wo_hbm, wo_v, s_wo.at[0])

    cp_x(0).start()
    cp_wq.start()
    cp_bx(0).start()
    cp_wk(0).start()
    for t in range(1, NQ):
        cp_x(t).start()
        cp_bx(t).start()
        cp_wk(t).start()
    cp_wv.start()
    cp_wo.start()
    for c in range(NO):
        cp_wg(c).start()
        cp_wu(c).start()
        cp_wd(c).start()

    cp_wq.wait()
    w_r = wr_ref[...].astype(F32)
    g_w = gw_ref[...].astype(F32)

    def q_step(t, carry):
        best, best_i = carry
        cp_x(t).wait()
        cp_bx(t).wait()
        cp_wk(t).wait()
        xt = x_v[rows(t, TQ), :]
        q = jnp.dot(xt, wq_v[...], preferred_element_type=F32)
        pq_v[rows(t, TQ), :] = _phi(q).astype(BF16)
        g_v[rows(t, TQ), :] = jnp.broadcast_to(_sigmoid(_rowdot(xt, g_w)), (TQ, 128))
        wkt_v[rows(t, D // NQ), :] = wk_v[t].T
        r = _rbf(_rowdot(bx_v[rows(t, TQ), :], w_r))
        r = jnp.where(r != r, -jnp.inf, r)
        m = jnp.max(r, axis=0, keepdims=True)
        ids = lax.broadcasted_iota(jnp.int32, (TQ, 1), 0) + t * TQ
        mi = jnp.min(jnp.where(r == m, ids, S), axis=0, keepdims=True)
        better = m > best
        return jnp.where(better, m, best), jnp.where(better, mi, best_i)

    best, best_i = lax.fori_loop(
        0, NQ, q_step, (jnp.full((1, 1), -jnp.inf, F32), jnp.zeros((1, 1), jnp.int32)))

    idx = jnp.clip(best_i[0, 0], 0, S - 1)
    grp = pl.multiple_of((idx // 16) * 16, 16)
    sel = lax.broadcasted_iota(jnp.int32, (16, 1), 0) == idx - grp
    b_grp = bx_v[pl.ds(grp, 16), :].astype(F32)
    x_sel = jnp.sum(jnp.where(sel, b_grp, 0.0), axis=0, keepdims=True)
    xcol_v[...] = _to_col(x_sel)

    cp_wv.wait()
    cp_wo.wait()
    same_head = (lax.broadcasted_iota(jnp.int32, (128, 128), 0) // DH
                 == lax.broadcasted_iota(jnp.int32, (128, 128), 1) // DH)

    def k_step(b, _):
        kt = lax.dot_general(wkt_v[rows(b, RK), :], x_v[...], (((1,), (1,)), ((), ())),
                             preferred_element_type=F32)
        pkt = _phi(kt).astype(BF16)
        pk32 = pkt.astype(F32)
        zacc = pk32[:, 0:128]
        for j in range(1, S // 128):
            zacc = zacc + pk32[:, j * 128:(j + 1) * 128]
        z = jnp.sum(zacc, axis=1, keepdims=True)
        gm = jnp.dot(pkt, x_v[...], preferred_element_type=F32).astype(BF16)
        for j in range(RK // 128):
            blk = rows(b * (RK // 128) + j, 128)
            kv = jnp.dot(gm[j * 128:(j + 1) * 128, :], wv_v[:, blk], preferred_element_type=F32)
            kv = jnp.where(same_head, kv, 0.0).astype(BF16)
            m_v[blk, :] = jnp.dot(kv, wo_v[blk, :], preferred_element_type=F32).astype(BF16)
            z_v[blk, :] = jnp.where(same_head, z[j * 128:(j + 1) * 128, :], 0.0).astype(BF16)
        return 0

    lax.fori_loop(0, NK, k_step, 0)

    t_sel = idx // TO
    loc = pl.multiple_of(grp - t_sel * TO, 16)

    def o_step(i, y):
        t = (t_sel + 1 + i) % NO
        cp_wg(i).wait()
        cp_wu(i).wait()
        cp_wd(i).wait()
        pq = pq_v[rows(t, TO), :]
        den = jnp.concatenate(
            [jnp.dot(pq[:, j * 128:(j + 1) * 128], z_v[j * 128:(j + 1) * 128, :],
                     preferred_element_type=F32) for j in range(D // 128)], axis=1) + 1e-6
        pqn = (pq.astype(F32) / den).astype(BF16)
        a = jnp.dot(pqn, m_v[...], preferred_element_type=F32)
        asel_v[...] = a
        g = jnp.tile(g_v[rows(t, TO), :], (1, D // 128))
        bt = bx_v[rows(t, TO), :].astype(F32)
        o_v[rows(t, TO), :] = (g * a + (1.0 - g) * (bt + bt * 0.0)).astype(BF16)

        ga = jnp.zeros((8, FC), F32)
        ua = jnp.zeros((8, FC), F32)
        for k in range(D // 16):
            xc = xcol_v[k * 16:(k + 1) * 16, :]
            xc = jnp.tile(xc, (1, FC // 128))
            pg = wg_v[i, k * 16:(k + 1) * 16, :].astype(F32) * xc
            pu = wu_v[i, k * 16:(k + 1) * 16, :].astype(F32) * xc
            ga = ga + pg[0:8] + pg[8:16]
            ua = ua + pu[0:8] + pu[8:16]
        gate = _rbf(jnp.sum(ga, axis=0, keepdims=True))
        up = _rbf(jnp.sum(ua, axis=0, keepdims=True))
        hcol = _to_col(_rbf(_rbf(gate * _sigmoid(gate)) * up))
        for k in range(FC // 16):
            hc = jnp.tile(hcol[k * 16:(k + 1) * 16, :], (1, D // 128))
            pd = wd_v[i, k * 16:(k + 1) * 16, :].astype(F32) * hc
            y = y + pd[0:8] + pd[8:16]

        @pl.when(i < NO - 1)
        def _():
            cp_o(t, i).start()
        return y

    y = lax.fori_loop(0, NO, o_step, jnp.zeros((8, D), F32))

    y = _rbf(_rbf(jnp.sum(y, axis=0, keepdims=True)) * _rbf(_sigmoid(best)))
    g = jnp.tile(g_v[pl.ds(grp, 16), :], (1, D // 128))
    b_new = b_grp + (b_grp * 0.0 + jnp.where(sel, y, 0.0))
    o_v[pl.ds(grp, 16), :] = (g * asel_v[pl.ds(loc, 16), :] + (1.0 - g) * b_new).astype(BF16)
    cp_o(t_sel, NO - 1).start()
    for i in range(NO):
        cp_o(0, i).wait()


@jax.jit
def pallas_gated_mix__linear_attn_block__moe_arch_mod__prompt_kernel(
    A_x: jax.Array,
    A_wqkv: jax.Array,
    A_wo: jax.Array,
    B_x: jax.Array,
    B_w_r: jax.Array,
    B_w_gate: jax.Array,
    B_w_up: jax.Array,
    B_w_down: jax.Array,
    gate_w: jax.Array,
):
    hbm = pl.BlockSpec(memory_space=pl.ANY)
    vmem = pl.BlockSpec(memory_space=pltpu.VMEM)
    dma = pltpu.SemaphoreType.DMA
    out = pl.pallas_call(
        _kernel,
        out_shape=jax.ShapeDtypeStruct((S, D), BF16),
        in_specs=[hbm, hbm, hbm, hbm, vmem, hbm, hbm, hbm, vmem],
        out_specs=hbm,
        scratch_shapes=[
            pltpu.VMEM((S, D), BF16),
            pltpu.VMEM((S, D), BF16),
            pltpu.VMEM((D, D), BF16),
            pltpu.VMEM((NQ, D, D // NQ), BF16),
            pltpu.VMEM((D, D), BF16),
            pltpu.VMEM((D, D), BF16),
            pltpu.VMEM((NO, D, FC), BF16),
            pltpu.VMEM((NO, D, FC), BF16),
            pltpu.VMEM((NO, FC, D), BF16),
            pltpu.VMEM((S, D), BF16),
            pltpu.VMEM((D, D), BF16),
            pltpu.VMEM((D, D), BF16),
            pltpu.VMEM((D, 128), BF16),
            pltpu.VMEM((S, 128), F32),
            pltpu.VMEM((D, 128), F32),
            pltpu.VMEM((S, D), BF16),
            pltpu.VMEM((TO, D), F32),
            dma((NQ,)), dma((NQ,)), dma((1,)), dma((NQ,)), dma((1,)), dma((1,)),
            dma((NO,)), dma((NO,)), dma((NO,)), dma((NO,)),
        ],
        compiler_params=pltpu.CompilerParams(vmem_limit_bytes=100 * 1024 * 1024),
    )(A_x.reshape(S, D), A_wqkv, A_wo, B_x.reshape(S, D), B_w_r.reshape(1, D),
      B_w_gate, B_w_up, B_w_down, gate_w.reshape(1, D))
    return out.reshape(1, S, D)
```

```python
import jax
import jax.numpy as jnp
from jax import lax
import jax.experimental.pallas as pl
import jax.experimental.pallas.tpu as pltpu

S, D, F, H = 2048, 1024, 3584, 32
DH = D // H
TQ = 512
RK = 256
TO = 512
NQ, NK, NO = S // TQ, D // RK, S // TO
FC = F // NO
F32, BF16 = jnp.float32, jnp.bfloat16


def _phi(t):
    return jnp.where(t > 0, t + 1.0, jnp.exp(t)) + 1e-6


def _sigmoid(t):
    return 1.0 / (1.0 + jnp.exp(-t))


def _rbf(t):
    return t.astype(BF16).astype(F32)


def _rowdot(a, w):
    acc = a[:, 0:128].astype(F32) * w[:, 0:128]
    for j in range(1, D // 128):
        acc = acc + a[:, j * 128:(j + 1) * 128].astype(F32) * w[:, j * 128:(j + 1) * 128]
    return jnp.sum(acc, axis=1, keepdims=True)


def _to_col(row):
    return jnp.broadcast_to(row, (128, row.shape[1])).T


def _kernel(x_hbm, wqkv_hbm, wo_hbm, bx_hbm, wr_ref, wg_hbm, wu_hbm, wd_hbm, gw_ref,
            o_hbm,
            x_v, bx_v, wq_v, wk_v, wv_v, wo_v, wg_v, wu_v, wd_v,
            pq_v, wkt_v, m_v, z_v, g_v, xcol_v, o_v, asel_v,
            s_x, s_bx, s_wq, s_wk, s_wv, s_wo, s_wg, s_wu, s_wd, s_o):

    def rows(i, n):
        return pl.ds(pl.multiple_of(i * n, n), n)

    def cp_x(t):
        return pltpu.make_async_copy(x_hbm.at[rows(t, TQ)], x_v.at[rows(t, TQ)], s_x.at[t])

    def cp_bx(t):
        return pltpu.make_async_copy(bx_hbm.at[rows(t, TQ)], bx_v.at[rows(t, TQ)], s_bx.at[t])

    def cp_wk(t):
        n = D // NQ
        return pltpu.make_async_copy(wqkv_hbm.at[:, pl.ds(pl.multiple_of(D + t * n, n), n)],
                                     wk_v.at[t], s_wk.at[t])

    def cp_wg(c):
        return pltpu.make_async_copy(wg_hbm.at[:, rows(c, FC)], wg_v.at[c], s_wg.at[c])

    def cp_wu(c):
        return pltpu.make_async_copy(wu_hbm.at[:, rows(c, FC)], wu_v.at[c], s_wu.at[c])

    def cp_wd(c):
        return pltpu.make_async_copy(wd_hbm.at[rows(c, FC)], wd_v.at[c], s_wd.at[c])

    def cp_o(t, slot):
        return pltpu.make_async_copy(o_v.at[rows(t, TO)], o_hbm.at[rows(t, TO)], s_o.at[slot])

    cp_wq = pltpu.make_async_copy(wqkv_hbm.at[:, 0:D], wq_v, s_wq.at[0])
    cp_wv = pltpu.make_async_copy(wqkv_hbm.at[:, 2 * D:3 * D], wv_v, s_wv.at[0])
    cp_wo = pltpu.make_async_copy(wo_hbm, wo_v, s_wo.at[0])

    cp_x(0).start()
    cp_wq.start()
    cp_bx(0).start()
    cp_wk(0).start()

    cp_wq.wait()
    w_r = wr_ref[...].astype(F32)
    g_w = gw_ref[...].astype(F32)

    def q_step(t, carry):
        best, best_i = carry
        @pl.when(t + 1 < NQ)
        def _():
            cp_x(t + 1).start()
            cp_bx(t + 1).start()
            cp_wk(t + 1).start()

        @pl.when(t == NQ - 2)
        def _():
            cp_wv.start()

        @pl.when(t == NQ - 1)
        def _():
            cp_wo.start()

        cp_x(t).wait()
        cp_bx(t).wait()
        cp_wk(t).wait()
        xt = x_v[rows(t, TQ), :]
        q = jnp.dot(xt, wq_v[...], preferred_element_type=F32)
        pq_v[rows(t, TQ), :] = _phi(q).astype(BF16)
        g_v[rows(t, TQ), :] = jnp.broadcast_to(_sigmoid(_rowdot(xt, g_w)), (TQ, 128))
        wkt_v[rows(t, D // NQ), :] = wk_v[t].T
        r = _rbf(_rowdot(bx_v[rows(t, TQ), :], w_r))
        r = jnp.where(r != r, -jnp.inf, r)
        m = jnp.max(r, axis=0, keepdims=True)
        ids = lax.broadcasted_iota(jnp.int32, (TQ, 1), 0) + t * TQ
        mi = jnp.min(jnp.where(r == m, ids, S), axis=0, keepdims=True)
        better = m > best
        return jnp.where(better, m, best), jnp.where(better, mi, best_i)

    best, best_i = lax.fori_loop(
        0, NQ, q_step, (jnp.full((1, 1), -jnp.inf, F32), jnp.zeros((1, 1), jnp.int32)))

    idx = jnp.clip(best_i[0, 0], 0, S - 1)
    grp = pl.multiple_of((idx // 16) * 16, 16)
    sel = lax.broadcasted_iota(jnp.int32, (16, 1), 0) == idx - grp
    b_grp = bx_v[pl.ds(grp, 16), :].astype(F32)
    x_sel = jnp.sum(jnp.where(sel, b_grp, 0.0), axis=0, keepdims=True)
    xcol_v[...] = _to_col(x_sel)

    cp_wv.wait()
    cp_wo.wait()
    same_head = (lax.broadcasted_iota(jnp.int32, (128, 128), 0) // DH
                 == lax.broadcasted_iota(jnp.int32, (128, 128), 1) // DH)

    def k_step(b, _):
        cp_wg(b).start()
        cp_wu(b).start()
        cp_wd(b).start()
        kt = lax.dot_general(wkt_v[rows(b, RK), :], x_v[...], (((1,), (1,)), ((), ())),
                             preferred_element_type=F32)
        pkt = _phi(kt).astype(BF16)
        pk32 = pkt.astype(F32)
        zacc = pk32[:, 0:128]
        for j in range(1, S // 128):
            zacc = zacc + pk32[:, j * 128:(j + 1) * 128]
        z = jnp.sum(zacc, axis=1, keepdims=True)
        gm = jnp.dot(pkt, x_v[...], preferred_element_type=F32).astype(BF16)
        for j in range(RK // 128):
            blk = rows(b * (RK // 128) + j, 128)
            kv = jnp.dot(gm[j * 128:(j + 1) * 128, :], wv_v[:, blk], preferred_element_type=F32)
            kv = jnp.where(same_head, kv, 0.0).astype(BF16)
            m_v[blk, :] = jnp.dot(kv, wo_v[blk, :], preferred_element_type=F32).astype(BF16)
            z_v[blk, :] = jnp.where(same_head, z[j * 128:(j + 1) * 128, :], 0.0).astype(BF16)
        return 0

    lax.fori_loop(0, NK, k_step, 0)

    t_sel = idx // TO
    loc = pl.multiple_of(grp - t_sel * TO, 16)

    def o_step(i, y):
        t = (t_sel + 1 + i) % NO
        cp_wg(i).wait()
        cp_wu(i).wait()
        cp_wd(i).wait()
        pq = pq_v[rows(t, TO), :]
        den = jnp.concatenate(
            [jnp.dot(pq[:, j * 128:(j + 1) * 128], z_v[j * 128:(j + 1) * 128, :],
                     preferred_element_type=F32) for j in range(D // 128)], axis=1) + 1e-6
        pqn = (pq.astype(F32) / den).astype(BF16)
        a = jnp.dot(pqn, m_v[...], preferred_element_type=F32)
        asel_v[...] = a
        g = jnp.tile(g_v[rows(t, TO), :], (1, D // 128))
        bt = bx_v[rows(t, TO), :].astype(F32)
        o_v[rows(t, TO), :] = (g * a + (1.0 - g) * (bt + bt * 0.0)).astype(BF16)

        ga = jnp.zeros((8, FC), F32)
        ua = jnp.zeros((8, FC), F32)
        for k in range(D // 16):
            xc = xcol_v[k * 16:(k + 1) * 16, :]
            xc = jnp.tile(xc, (1, FC // 128))
            pg = wg_v[i, k * 16:(k + 1) * 16, :].astype(F32) * xc
            pu = wu_v[i, k * 16:(k + 1) * 16, :].astype(F32) * xc
            ga = ga + pg[0:8] + pg[8:16]
            ua = ua + pu[0:8] + pu[8:16]
        gate = _rbf(jnp.sum(ga, axis=0, keepdims=True))
        up = _rbf(jnp.sum(ua, axis=0, keepdims=True))
        hcol = _to_col(_rbf(_rbf(gate * _sigmoid(gate)) * up))
        for k in range(FC // 16):
            hc = jnp.tile(hcol[k * 16:(k + 1) * 16, :], (1, D // 128))
            pd = wd_v[i, k * 16:(k + 1) * 16, :].astype(F32) * hc
            y = y + pd[0:8] + pd[8:16]

        @pl.when(i < NO - 1)
        def _():
            cp_o(t, i).start()
        return y

    y = lax.fori_loop(0, NO, o_step, jnp.zeros((8, D), F32))

    y = _rbf(_rbf(jnp.sum(y, axis=0, keepdims=True)) * _rbf(_sigmoid(best)))
    g = jnp.tile(g_v[pl.ds(grp, 16), :], (1, D // 128))
    b_new = b_grp + (b_grp * 0.0 + jnp.where(sel, y, 0.0))
    o_v[pl.ds(grp, 16), :] = (g * asel_v[pl.ds(loc, 16), :] + (1.0 - g) * b_new).astype(BF16)
    cp_o(t_sel, NO - 1).start()
    for i in range(NO):
        cp_o(0, i).wait()


@jax.jit
def pallas_gated_mix__linear_attn_block__moe_arch_mod__prompt_kernel(
    A_x: jax.Array,
    A_wqkv: jax.Array,
    A_wo: jax.Array,
    B_x: jax.Array,
    B_w_r: jax.Array,
    B_w_gate: jax.Array,
    B_w_up: jax.Array,
    B_w_down: jax.Array,
    gate_w: jax.Array,
):
    hbm = pl.BlockSpec(memory_space=pl.ANY)
    vmem = pl.BlockSpec(memory_space=pltpu.VMEM)
    dma = pltpu.SemaphoreType.DMA
    out = pl.pallas_call(
        _kernel,
        out_shape=jax.ShapeDtypeStruct((S, D), BF16),
        in_specs=[hbm, hbm, hbm, hbm, vmem, hbm, hbm, hbm, vmem],
        out_specs=hbm,
        scratch_shapes=[
            pltpu.VMEM((S, D), BF16),
            pltpu.VMEM((S, D), BF16),
            pltpu.VMEM((D, D), BF16),
            pltpu.VMEM((NQ, D, D // NQ), BF16),
            pltpu.VMEM((D, D), BF16),
            pltpu.VMEM((D, D), BF16),
            pltpu.VMEM((NO, D, FC), BF16),
            pltpu.VMEM((NO, D, FC), BF16),
            pltpu.VMEM((NO, FC, D), BF16),
            pltpu.VMEM((S, D), BF16),
            pltpu.VMEM((D, D), BF16),
            pltpu.VMEM((D, D), BF16),
            pltpu.VMEM((D, 128), BF16),
            pltpu.VMEM((S, 128), F32),
            pltpu.VMEM((D, 128), F32),
            pltpu.VMEM((S, D), BF16),
            pltpu.VMEM((TO, D), F32),
            dma((NQ,)), dma((NQ,)), dma((1,)), dma((NQ,)), dma((1,)), dma((1,)),
            dma((NO,)), dma((NO,)), dma((NO,)), dma((NO,)),
        ],
        compiler_params=pltpu.CompilerParams(vmem_limit_bytes=100 * 1024 * 1024),
    )(A_x.reshape(S, D), A_wqkv, A_wo, B_x.reshape(S, D), B_w_r.reshape(1, D),
      B_w_gate, B_w_up, B_w_down, gate_w.reshape(1, D))
    return out.reshape(1, S, D)
```

```python
import jax
import jax.numpy as jnp
from jax import lax
import jax.experimental.pallas as pl
import jax.experimental.pallas.tpu as pltpu

S, D, F, H = 2048, 1024, 3584, 32
DH = D // H
RK = 256
TO = 512
NK, NO = D // RK, S // TO
NF = 3
F_CHUNKS = ((0, 1280), (1280, 2432), (2432, 3584))
X_CHUNKS = ((0, 512), (512, 1024), (1024, 2048))
F32, BF16 = jnp.float32, jnp.bfloat16


def _phi(t):
    return jnp.where(t > 0, t + 1.0, jnp.exp(t)) + 1e-6


def _sigmoid(t):
    return 1.0 / (1.0 + jnp.exp(-t))


def _rbf(t):
    return t.astype(BF16).astype(F32)


def _rowdot(a, w):
    acc = a[:, 0:128].astype(F32) * w[:, 0:128]
    for j in range(1, D // 128):
        acc = acc + a[:, j * 128:(j + 1) * 128].astype(F32) * w[:, j * 128:(j + 1) * 128]
    return jnp.sum(acc, axis=1, keepdims=True)


def _to_col(row):
    return jnp.broadcast_to(row, (128, row.shape[1])).T


def _kernel(x_hbm, wqkv_hbm, wo_hbm, bx_hbm, wr_ref, wg_hbm, wu_hbm, wd_hbm, gw_ref,
            o_hbm,
            x_v, bx_v, wq_v, wk_v, wv_v, wo_v, wg_v, wu_v, wd_v,
            pqn_v, m_v, g_v, xcol_v, o_v, a_v,
            s_x, s_bx, s_wq, s_wk, s_wv, s_wo, s_wg, s_wu, s_wd, s_o):
    copy = pltpu.make_async_copy

    def blk(i, n):
        return slice(i * n, (i + 1) * n)

    cp_x = [copy(x_hbm.at[lo:hi], x_v.at[lo:hi], s_x.at[i]) for i, (lo, hi) in enumerate(X_CHUNKS)]
    cp_bx = [copy(bx_hbm.at[blk(t, TO)], bx_v.at[blk(t, TO)], s_bx.at[t]) for t in range(NO)]
    cp_wq = [copy(wqkv_hbm.at[:, blk(b, RK)], wq_v.at[b], s_wq.at[b]) for b in range(NK)]
    cp_wk = [copy(wqkv_hbm.at[:, blk(NK + b, RK)], wk_v.at[b], s_wk.at[b]) for b in range(NK)]
    cp_wv = [copy(wqkv_hbm.at[:, blk(2 * NK + b, RK)], wv_v.at[b], s_wv.at[b]) for b in range(NK)]
    cp_wo = [copy(wo_hbm.at[blk(b, RK)], wo_v.at[blk(b, RK)], s_wo.at[b]) for b in range(NK)]
    cp_wg = [copy(wg_hbm.at[:, lo:hi], wg_v.at[:, lo:hi], s_wg.at[c]) for c, (lo, hi) in enumerate(F_CHUNKS)]
    cp_wu = [copy(wu_hbm.at[:, lo:hi], wu_v.at[:, lo:hi], s_wu.at[c]) for c, (lo, hi) in enumerate(F_CHUNKS)]
    cp_wd = [copy(wd_hbm.at[lo:hi], wd_v.at[lo:hi], s_wd.at[c]) for c, (lo, hi) in enumerate(F_CHUNKS)]

    def start(*cps):
        for c in cps:
            c.start()

    def wait(*cps):
        for c in cps:
            c.wait()

    w_r = wr_ref[...].astype(F32).reshape(1, D)
    g_w = gw_ref[...].astype(F32).reshape(1, D)
    same_head = (lax.broadcasted_iota(jnp.int32, (128, 128), 0) // DH
                 == lax.broadcasted_iota(jnp.int32, (128, 128), 1) // DH)

    def kq_weights(b):
        return jnp.concatenate([wk_v[b].T, wq_v[b].T], axis=0)

    def kq_proj(wt, lo, hi):
        t = lax.dot_general(wt, x_v[lo:hi, :], (((1,), (1,)), ((), ())), preferred_element_type=F32)
        return _phi(t).astype(BF16)

    def k_step(b, p):
        pk = p[0:RK]
        pk32 = pk.astype(F32)
        zacc = pk32[:, 0:128]
        for j in range(1, S // 128):
            zacc = zacc + pk32[:, blk(j, 128)]
        z = _rbf(jnp.sum(zacc, axis=1, keepdims=True))
        gm = jnp.dot(pk, x_v[...], preferred_element_type=F32).astype(BF16)
        for j in range(RK // 128):
            rows = blk(b * (RK // 128) + j, 128)
            kv = jnp.dot(gm[blk(j, 128)], wv_v[b, :, blk(j, 128)], preferred_element_type=F32)
            kv = jnp.where(same_head, kv, 0.0).astype(BF16)
            m_v[rows, :] = jnp.dot(kv, wo_v[rows, :], preferred_element_type=F32).astype(BF16)
        pqn = []
        for h in range(RK // DH):
            pq = p[RK + h * DH:RK + (h + 1) * DH].astype(F32)
            den = jnp.sum(pq * z[blk(h, DH)], axis=0, keepdims=True) + 1e-6
            pqn.append((pq * (1.0 / den)).astype(BF16))
        pqn_v[:, blk(b, RK)] = jnp.concatenate(pqn, axis=0).T

    def route_step(t, best, best_i):
        g_v[blk(t, TO), :] = jnp.broadcast_to(_sigmoid(_rowdot(x_v[blk(t, TO), :], g_w)), (TO, 128))
        r = _rbf(_rowdot(bx_v[blk(t, TO), :], w_r))
        r = jnp.where(r != r, -jnp.inf, r)
        m = jnp.max(r, axis=0, keepdims=True)
        ids = lax.broadcasted_iota(jnp.int32, (TO, 1), 0) + t * TO
        mi = jnp.min(jnp.where(r == m, ids, S), axis=0, keepdims=True)
        better = m > best
        return jnp.where(better, m, best), jnp.where(better, mi, best_i)

    def ffn_step(c, y):
        lo, hi = F_CHUNKS[c]
        ga = jnp.zeros((8, hi - lo), F32)
        ua = jnp.zeros((8, hi - lo), F32)
        for k in range(D // 16):
            xc = jnp.tile(xcol_v[blk(k, 16), :], (1, (hi - lo) // 128))
            pg = wg_v[blk(k, 16), lo:hi].astype(F32) * xc
            pu = wu_v[blk(k, 16), lo:hi].astype(F32) * xc
            ga = ga + pg[0:8] + pg[8:16]
            ua = ua + pu[0:8] + pu[8:16]
        gate = _rbf(jnp.sum(ga, axis=0, keepdims=True))
        up = _rbf(jnp.sum(ua, axis=0, keepdims=True))
        hcol = _to_col(_rbf(_rbf(gate * _sigmoid(gate)) * up))
        for k in range((hi - lo) // 16):
            pd = wd_v[lo + k * 16:lo + (k + 1) * 16, :].astype(F32) * jnp.tile(hcol[blk(k, 16)], (1, D // 128))
            y = y + pd[0:8] + pd[8:16]
        return y

    start(cp_wk[0], cp_wq[0], cp_x[0])
    wait(cp_wk[0], cp_wq[0])
    start(cp_x[1])
    wt = kq_weights(0)
    parts = []
    for i, (lo, hi) in enumerate(X_CHUNKS):
        if i + 2 < len(X_CHUNKS):
            start(cp_x[i + 2])
        elif i + 2 == len(X_CHUNKS):
            start(cp_wv[0], cp_wo[0], cp_wk[1], cp_wq[1])
        else:
            start(cp_bx[0], cp_bx[1])
        wait(cp_x[i])
        parts.append(kq_proj(wt, lo, hi))
    p = jnp.concatenate(parts, axis=1)

    best = jnp.full((1, 1), -jnp.inf, F32)
    best_i = jnp.zeros((1, 1), jnp.int32)
    for b in range(NK):
        if b == 0:
            start(cp_bx[2], cp_bx[3], cp_wv[1], cp_wo[1], cp_wk[2], cp_wq[2])
            wait(cp_wv[0], cp_wo[0], cp_wk[1], cp_wq[1], cp_bx[0], cp_bx[1])
        elif b == 1:
            start(cp_wv[2], cp_wo[2], cp_wk[3], cp_wq[3], cp_wg[0], cp_wu[0], cp_wd[0])
            wait(cp_wv[1], cp_wo[1], cp_wk[2], cp_wq[2], cp_bx[2], cp_bx[3])
        elif b == 2:
            start(cp_wv[3], cp_wo[3], cp_wg[1], cp_wu[1], cp_wd[1])
            wait(cp_wv[2], cp_wo[2], cp_wk[3], cp_wq[3])
        else:
            start(cp_wg[2], cp_wu[2], cp_wd[2])
            wait(cp_wv[3], cp_wo[3])
        if b > 0:
            p = kq_proj(wt, 0, S)
        k_step(b, p)
        if b + 1 < NK:
            wt = kq_weights(b + 1)
        if b < 2:
            for t in (2 * b, 2 * b + 1):
                best, best_i = route_step(t, best, best_i)
        if b == 2:
            idx = jnp.clip(best_i[0, 0], 0, S - 1)
            grp = pl.multiple_of((idx // 16) * 16, 16)
            sel = lax.broadcasted_iota(jnp.int32, (16, 1), 0) == idx - grp
            b_grp = bx_v[pl.ds(grp, 16), :].astype(F32)
            xcol_v[...] = _to_col(jnp.sum(jnp.where(sel, b_grp, 0.0), axis=0, keepdims=True))

    t_sel = idx // TO
    cp_o = [copy(o_v.at[blk(t, TO)], o_hbm.at[blk(t, TO)], s_o.at[t]) for t in range(NO)]
    cp_fix = copy(o_v.at[pl.ds(grp, 16)], o_hbm.at[pl.ds(grp, 16)], s_o.at[NO])
    y = jnp.zeros((8, D), F32)
    for t in range(NO):
        if t < NF:
            wait(cp_wg[t], cp_wu[t], cp_wd[t])
        a = jnp.dot(pqn_v[blk(t, TO), :], m_v[...], preferred_element_type=F32)
        a_v[(t_sel == t).astype(jnp.int32)] = a
        g = jnp.tile(g_v[blk(t, TO), :], (1, D // 128))
        bt = bx_v[blk(t, TO), :].astype(F32)
        o_v[blk(t, TO), :] = (g * a + (1.0 - g) * (bt + bt * 0.0)).astype(BF16)
        if t < NF:
            y = ffn_step(t, y)
        if t < NO - 1:
            cp_o[t].start()

    y = _rbf(_rbf(jnp.sum(y, axis=0, keepdims=True)) * _rbf(_sigmoid(best)))
    g = jnp.tile(g_v[pl.ds(grp, 16), :], (1, D // 128))
    a = a_v[1, pl.ds(pl.multiple_of(grp - t_sel * TO, 16), 16), :]
    b_new = b_grp + (b_grp * 0.0 + jnp.where(sel, y, 0.0))
    wait(*cp_o[:NO - 1])
    o_v[pl.ds(grp, 16), :] = (g * a + (1.0 - g) * b_new).astype(BF16)
    cp_o[NO - 1].start()

    @pl.when(t_sel < NO - 1)
    def _():
        cp_fix.start()
        cp_fix.wait()

    cp_o[NO - 1].wait()


@jax.jit
def pallas_gated_mix__linear_attn_block__moe_arch_mod__prompt_kernel(
    A_x: jax.Array,
    A_wqkv: jax.Array,
    A_wo: jax.Array,
    B_x: jax.Array,
    B_w_r: jax.Array,
    B_w_gate: jax.Array,
    B_w_up: jax.Array,
    B_w_down: jax.Array,
    gate_w: jax.Array,
):
    hbm = pl.BlockSpec(memory_space=pl.ANY)
    vmem = pl.BlockSpec(memory_space=pltpu.VMEM)
    dma = pltpu.SemaphoreType.DMA
    out = pl.pallas_call(
        _kernel,
        out_shape=jax.ShapeDtypeStruct((S, D), BF16),
        in_specs=[hbm, hbm, hbm, hbm, vmem, hbm, hbm, hbm, vmem],
        out_specs=hbm,
        scratch_shapes=[
            pltpu.VMEM((S, D), BF16),
            pltpu.VMEM((S, D), BF16),
            pltpu.VMEM((NK, D, RK), BF16),
            pltpu.VMEM((NK, D, RK), BF16),
            pltpu.VMEM((NK, D, RK), BF16),
            pltpu.VMEM((D, D), BF16),
            pltpu.VMEM((D, F), BF16),
            pltpu.VMEM((D, F), BF16),
            pltpu.VMEM((F, D), BF16),
            pltpu.VMEM((S, D), BF16),
            pltpu.VMEM((D, D), BF16),
            pltpu.VMEM((S, 128), F32),
            pltpu.VMEM((D, 128), F32),
            pltpu.VMEM((S, D), BF16),
            pltpu.VMEM((2, TO, D), F32),
            dma((len(X_CHUNKS),)), dma((NO,)), dma((NK,)), dma((NK,)), dma((NK,)), dma((NK,)),
            dma((NF,)), dma((NF,)), dma((NF,)), dma((NO + 1,)),
        ],
        compiler_params=pltpu.CompilerParams(vmem_limit_bytes=100 * 1024 * 1024),
    )(A_x.reshape(S, D), A_wqkv, A_wo, B_x.reshape(S, D), B_w_r,
      B_w_gate, B_w_up, B_w_down, gate_w)
    return out.reshape(1, S, D)
```

```python
import jax
import jax.numpy as jnp
from jax import lax
import jax.experimental.pallas as pl
import jax.experimental.pallas.tpu as pltpu

S, D, F, H = 2048, 1024, 3584, 32
DH = D // H
RK = 256
TO = 512
NK, NO = D // RK, S // TO
NF = 3
F_CHUNKS = ((0, 1280), (1280, 2432), (2432, 3584))
KQ_N, G_N, O_N = 256, 256, 256
RT = 128
FN = 128
X_CHUNKS = ((0, 512), (512, 1024), (1024, 2048))
F32, BF16 = jnp.float32, jnp.bfloat16


def _phi(t):
    return jnp.where(t > 0, t + 1.0, jnp.exp(t)) + 1e-6


def _sigmoid(t):
    return 1.0 / (1.0 + jnp.exp(-t))


def _rbf(t):
    return t.astype(BF16).astype(F32)


def _rowdot(a, w):
    acc = a[:, 0:128].astype(F32) * w[:, 0:128]
    for j in range(1, D // 128):
        acc = acc + a[:, j * 128:(j + 1) * 128].astype(F32) * w[:, j * 128:(j + 1) * 128]
    return jnp.sum(acc, axis=1, keepdims=True)


def _to_col(row):
    return jnp.broadcast_to(row, (128, row.shape[1])).T


def _kernel(x_hbm, wqkv_hbm, wo_hbm, bx_hbm, wr_ref, wg_hbm, wu_hbm, wd_hbm, gw_ref,
            o_hbm,
            x_v, bx_v, wq_v, wk_v, wv_v, wo_v, wg_v, wu_v, wd_v,
            pqn_v, m_v, g_v, xcol_v, o_v, a_v,
            s_x, s_bx, s_wq, s_wk, s_wv, s_wo, s_wg, s_wu, s_wd, s_o):
    copy = pltpu.make_async_copy

    def blk(i, n):
        return slice(i * n, (i + 1) * n)

    cp_x = [copy(x_hbm.at[lo:hi], x_v.at[lo:hi], s_x.at[i]) for i, (lo, hi) in enumerate(X_CHUNKS)]
    cp_bx = [copy(bx_hbm.at[blk(t, TO)], bx_v.at[blk(t, TO)], s_bx.at[t]) for t in range(NO)]
    cp_wq = [copy(wqkv_hbm.at[:, blk(b, RK)], wq_v.at[b], s_wq.at[b]) for b in range(NK)]
    cp_wk = [copy(wqkv_hbm.at[:, blk(NK + b, RK)], wk_v.at[b], s_wk.at[b]) for b in range(NK)]
    cp_wv = [copy(wqkv_hbm.at[:, blk(2 * NK + b, RK)], wv_v.at[b], s_wv.at[b]) for b in range(NK)]
    cp_wo = [copy(wo_hbm.at[blk(b, RK)], wo_v.at[blk(b, RK)], s_wo.at[b]) for b in range(NK)]
    cp_wg = [copy(wg_hbm.at[:, lo:hi], wg_v.at[:, lo:hi], s_wg.at[c]) for c, (lo, hi) in enumerate(F_CHUNKS)]
    cp_wu = [copy(wu_hbm.at[:, lo:hi], wu_v.at[:, lo:hi], s_wu.at[c]) for c, (lo, hi) in enumerate(F_CHUNKS)]
    cp_wd = [copy(wd_hbm.at[lo:hi], wd_v.at[lo:hi], s_wd.at[c]) for c, (lo, hi) in enumerate(F_CHUNKS)]

    def start(*cps):
        for c in cps:
            c.start()

    def wait(*cps):
        for c in cps:
            c.wait()

    w_r = wr_ref[...].astype(F32).reshape(1, D)
    g_w = gw_ref[...].astype(F32).reshape(1, D)
    same_head = (lax.broadcasted_iota(jnp.int32, (128, 128), 0) // DH
                 == lax.broadcasted_iota(jnp.int32, (128, 128), 1) // DH)

    def kq_weights(b):
        return jnp.concatenate([wk_v[b].T, wq_v[b].T], axis=0)

    def tick(bg, n=1):
        for _ in range(n):
            next(bg, None)

    def kq_proj(wt, lo, hi, bg):
        parts = []
        for c in range(lo, hi, KQ_N):
            t = lax.dot_general(wt, x_v[c:c + KQ_N, :], (((1,), (1,)), ((), ())),
                                preferred_element_type=F32)
            parts.append(_phi(t).astype(BF16))
            tick(bg)
        return parts

    def k_step(b, p, bg):
        pk = p[0:RK]
        pk32 = pk.astype(F32)
        zacc = pk32[:, 0:128]
        for j in range(1, S // 128):
            zacc = zacc + pk32[:, blk(j, 128)]
        z = _rbf(jnp.sum(zacc, axis=1, keepdims=True))
        gm = []
        for c in range(0, D, G_N):
            gm.append(jnp.dot(pk, x_v[:, c:c + G_N], preferred_element_type=F32).astype(BF16))
            tick(bg, G_N // 128)
        gm = jnp.concatenate(gm, axis=1)
        for j in range(RK // 128):
            rows = blk(b * (RK // 128) + j, 128)
            kv = jnp.dot(gm[blk(j, 128)], wv_v[b, :, blk(j, 128)], preferred_element_type=F32)
            kv = jnp.where(same_head, kv, 0.0).astype(BF16)
            m_v[rows, :] = jnp.dot(kv, wo_v[rows, :], preferred_element_type=F32).astype(BF16)
        pqn = []
        for h in range(RK // DH):
            pq = p[RK + h * DH:RK + (h + 1) * DH].astype(F32)
            den = jnp.sum(pq * z[blk(h, DH)], axis=0, keepdims=True) + 1e-6
            pqn.append((pq * (1.0 / den)).astype(BF16))
        pqn_v[:, blk(b, RK)] = jnp.concatenate(pqn, axis=0).T

    route = {"best": jnp.full((1, 1), -jnp.inf, F32), "idx": jnp.zeros((1, 1), jnp.int32)}

    def route_work(lo, hi):
        for t in range(lo, hi, RT):
            g_v[t:t + RT, :] = jnp.broadcast_to(_sigmoid(_rowdot(x_v[t:t + RT, :], g_w)), (RT, 128))
            r = _rbf(_rowdot(bx_v[t:t + RT, :], w_r))
            r = jnp.where(r != r, -jnp.inf, r)
            m = jnp.max(r, axis=0, keepdims=True)
            ids = lax.broadcasted_iota(jnp.int32, (RT, 1), 0) + t
            mi = jnp.min(jnp.where(r == m, ids, S), axis=0, keepdims=True)
            better = m > route["best"]
            route["best"] = jnp.where(better, m, route["best"])
            route["idx"] = jnp.where(better, mi, route["idx"])
            yield

    ffn = {"y": jnp.zeros((8, D), F32)}

    def ffn_work(lo, hi):
        for c in range(lo, hi, FN):
            ga = jnp.zeros((8, FN), F32)
            ua = jnp.zeros((8, FN), F32)
            for k in range(D // 16):
                xc = jnp.tile(xcol_v[blk(k, 16), :], (1, FN // 128))
                pg = wg_v[blk(k, 16), c:c + FN].astype(F32) * xc
                pu = wu_v[blk(k, 16), c:c + FN].astype(F32) * xc
                ga = ga + pg[0:8] + pg[8:16]
                ua = ua + pu[0:8] + pu[8:16]
            gate = _rbf(jnp.sum(ga, axis=0, keepdims=True))
            up = _rbf(jnp.sum(ua, axis=0, keepdims=True))
            hcol = _to_col(_rbf(_rbf(gate * _sigmoid(gate)) * up))
            y = ffn["y"]
            for k in range(FN // 16):
                pd = wd_v[c + k * 16:c + (k + 1) * 16, :].astype(F32) * jnp.tile(hcol[blk(k, 16)], (1, D // 128))
                y = y + pd[0:8] + pd[8:16]
            ffn["y"] = y
            yield

    start(cp_wk[0], cp_wq[0], cp_x[0])
    wait(cp_wk[0], cp_wq[0])
    start(cp_x[1])
    wt = kq_weights(0)
    parts = []
    for i, (lo, hi) in enumerate(X_CHUNKS):
        if i + 2 < len(X_CHUNKS):
            start(cp_x[i + 2])
        elif i + 2 == len(X_CHUNKS):
            start(cp_wv[0], cp_wo[0], cp_wk[1], cp_wq[1])
        else:
            start(cp_bx[0], cp_bx[1])
        wait(cp_x[i])
        parts += kq_proj(wt, lo, hi, iter(()))

    for b in range(NK):
        bg = route_work(b * S // 2, (b + 1) * S // 2) if b < 2 else iter(())
        if b == 0:
            start(cp_bx[2], cp_bx[3], cp_wv[1], cp_wo[1], cp_wk[2], cp_wq[2])
            wait(cp_wv[0], cp_wo[0], cp_wk[1], cp_wq[1], cp_bx[0], cp_bx[1])
        elif b == 1:
            start(cp_wv[2], cp_wo[2], cp_wk[3], cp_wq[3], cp_wg[0], cp_wu[0], cp_wd[0])
            wait(cp_wv[1], cp_wo[1], cp_wk[2], cp_wq[2], cp_bx[2], cp_bx[3])
        elif b == 2:
            start(cp_wv[3], cp_wo[3], cp_wg[1], cp_wu[1], cp_wd[1])
            wait(cp_wv[2], cp_wo[2], cp_wk[3], cp_wq[3])
        else:
            start(cp_wg[2], cp_wu[2], cp_wd[2])
            wait(cp_wv[3], cp_wo[3])
        if b > 0:
            parts = kq_proj(wt, 0, S, bg)
        k_step(b, jnp.concatenate(parts, axis=1), bg)
        tick(bg, S)
        if b + 1 < NK:
            wt = kq_weights(b + 1)
        if b == 2:
            idx = jnp.clip(route["idx"][0, 0], 0, S - 1)
            grp = pl.multiple_of((idx // 16) * 16, 16)
            sel = lax.broadcasted_iota(jnp.int32, (16, 1), 0) == idx - grp
            b_grp = bx_v[pl.ds(grp, 16), :].astype(F32)
            xcol_v[...] = _to_col(jnp.sum(jnp.where(sel, b_grp, 0.0), axis=0, keepdims=True))

    t_sel = idx // TO
    cp_o = [copy(o_v.at[blk(t, TO)], o_hbm.at[blk(t, TO)], s_o.at[t]) for t in range(NO)]
    cp_fix = copy(o_v.at[pl.ds(grp, 16)], o_hbm.at[pl.ds(grp, 16)], s_o.at[NO])
    for t in range(NO):
        bg = iter(())
        if t < NF:
            wait(cp_wg[t], cp_wu[t], cp_wd[t])
            bg = ffn_work(*F_CHUNKS[t])
        rows = blk(t, TO)
        slot = (t_sel == t).astype(jnp.int32)
        for c in range(0, D, O_N):
            a = jnp.dot(pqn_v[rows, :], m_v[:, c:c + O_N], preferred_element_type=F32)
            a_v[slot, :, c:c + O_N] = a
            g = jnp.tile(g_v[rows, :], (1, O_N // 128))
            bt = bx_v[rows, c:c + O_N].astype(F32)
            o_v[rows, c:c + O_N] = (g * a + (1.0 - g) * (bt + bt * 0.0)).astype(BF16)
            tick(bg, 3)
        tick(bg, F)
        if t < NO - 1:
            cp_o[t].start()

    y = _rbf(_rbf(jnp.sum(ffn["y"], axis=0, keepdims=True)) * _rbf(_sigmoid(route["best"])))
    g = jnp.tile(g_v[pl.ds(grp, 16), :], (1, D // 128))
    a = a_v[1, pl.ds(pl.multiple_of(grp - t_sel * TO, 16), 16), :]
    b_new = b_grp + (b_grp * 0.0 + jnp.where(sel, y, 0.0))
    wait(*cp_o[:NO - 1])
    o_v[pl.ds(grp, 16), :] = (g * a + (1.0 - g) * b_new).astype(BF16)
    cp_o[NO - 1].start()

    @pl.when(t_sel < NO - 1)
    def _():
        cp_fix.start()
        cp_fix.wait()

    cp_o[NO - 1].wait()


@jax.jit
def pallas_gated_mix__linear_attn_block__moe_arch_mod__prompt_kernel(
    A_x: jax.Array,
    A_wqkv: jax.Array,
    A_wo: jax.Array,
    B_x: jax.Array,
    B_w_r: jax.Array,
    B_w_gate: jax.Array,
    B_w_up: jax.Array,
    B_w_down: jax.Array,
    gate_w: jax.Array,
):
    hbm = pl.BlockSpec(memory_space=pl.ANY)
    vmem = pl.BlockSpec(memory_space=pltpu.VMEM)
    dma = pltpu.SemaphoreType.DMA
    out = pl.pallas_call(
        _kernel,
        out_shape=jax.ShapeDtypeStruct((S, D), BF16),
        in_specs=[hbm, hbm, hbm, hbm, vmem, hbm, hbm, hbm, vmem],
        out_specs=hbm,
        scratch_shapes=[
            pltpu.VMEM((S, D), BF16),
            pltpu.VMEM((S, D), BF16),
            pltpu.VMEM((NK, D, RK), BF16),
            pltpu.VMEM((NK, D, RK), BF16),
            pltpu.VMEM((NK, D, RK), BF16),
            pltpu.VMEM((D, D), BF16),
            pltpu.VMEM((D, F), BF16),
            pltpu.VMEM((D, F), BF16),
            pltpu.VMEM((F, D), BF16),
            pltpu.VMEM((S, D), BF16),
            pltpu.VMEM((D, D), BF16),
            pltpu.VMEM((S, 128), F32),
            pltpu.VMEM((D, 128), F32),
            pltpu.VMEM((S, D), BF16),
            pltpu.VMEM((2, TO, D), F32),
            dma((len(X_CHUNKS),)), dma((NO,)), dma((NK,)), dma((NK,)), dma((NK,)), dma((NK,)),
            dma((NF,)), dma((NF,)), dma((NF,)), dma((NO + 1,)),
        ],
        compiler_params=pltpu.CompilerParams(vmem_limit_bytes=100 * 1024 * 1024),
    )(A_x.reshape(S, D), A_wqkv, A_wo, B_x.reshape(S, D), B_w_r,
      B_w_gate, B_w_up, B_w_down, gate_w)
    return out.reshape(1, S, D)
```

```python
import jax
import jax.numpy as jnp
from jax import lax
import jax.experimental.pallas as pl
import jax.experimental.pallas.tpu as pltpu

S, D, F, H = 2048, 1024, 3584, 32
DH = D // H
RK = 256
TO = 512
NK, NO = D // RK, S // TO
F_CHUNKS = ((0, 1792), (1792, 3584))
NF = len(F_CHUNKS)
X_CHUNKS = ((0, 512), (512, 1024), (1024, 2048))
F32, BF16 = jnp.float32, jnp.bfloat16


def _phi(t):
    return jnp.where(t > 0, t + 1.0, jnp.exp(t)) + 1e-6


def _sigmoid(t):
    return 1.0 / (1.0 + jnp.exp(-t))


def _rbf(t):
    return t.astype(BF16).astype(F32)


def _rowdot(a, w):
    w = jnp.concatenate([w, w], axis=0)
    acc = a[:, 0:128].astype(F32) * w[:, 0:128]
    for j in range(1, D // 128):
        acc = acc + a[:, j * 128:(j + 1) * 128].astype(F32) * w[:, j * 128:(j + 1) * 128]
    return jnp.sum(acc, axis=1, keepdims=True)


def _to_col(row):
    return jnp.broadcast_to(row, (128, row.shape[1])).T


def _kernel(x_hbm, wqkv_hbm, wo_hbm, bx_hbm, wr_ref, wg_hbm, wu_hbm, wd_hbm, gw_ref,
            o_hbm,
            x_v, bx_v, wq_v, wk_v, wv_v, wo_v, wg_v, wu_v, wd_v,
            pqn_v, m_v, g_v, xcol_v, o_v, a_v,
            s_x, s_bx, s_wq, s_wk, s_wv, s_wo, s_wg, s_wu, s_wd, s_o):
    copy = pltpu.make_async_copy

    def blk(i, n):
        return slice(i * n, (i + 1) * n)

    cp_x = [copy(x_hbm.at[lo:hi], x_v.at[lo:hi], s_x.at[i]) for i, (lo, hi) in enumerate(X_CHUNKS)]
    cp_bx = [copy(bx_hbm.at[blk(t, TO)], bx_v.at[blk(t, TO)], s_bx.at[t]) for t in range(NO)]
    cp_wq = [copy(wqkv_hbm.at[:, blk(b, RK)], wq_v.at[b], s_wq.at[b]) for b in range(NK)]
    cp_wk = [copy(wqkv_hbm.at[:, blk(NK + b, RK)], wk_v.at[b], s_wk.at[b]) for b in range(NK)]
    cp_wv = [copy(wqkv_hbm.at[:, blk(2 * NK + b, RK)], wv_v.at[b], s_wv.at[b]) for b in range(NK)]
    cp_wo = [copy(wo_hbm.at[blk(b, RK)], wo_v.at[blk(b, RK)], s_wo.at[b]) for b in range(NK)]
    cp_wg = [copy(wg_hbm.at[:, lo:hi], wg_v.at[:, lo:hi], s_wg.at[c]) for c, (lo, hi) in enumerate(F_CHUNKS)]
    cp_wu = [copy(wu_hbm.at[:, lo:hi], wu_v.at[:, lo:hi], s_wu.at[c]) for c, (lo, hi) in enumerate(F_CHUNKS)]
    cp_wd = [copy(wd_hbm.at[lo:hi], wd_v.at[lo:hi], s_wd.at[c]) for c, (lo, hi) in enumerate(F_CHUNKS)]

    def start(*cps):
        for c in cps:
            c.start()

    def wait(*cps):
        for c in cps:
            c.wait()

    w_r = wr_ref[...].astype(F32).reshape(1, D)
    g_w = gw_ref[...].astype(F32).reshape(1, D)
    same_head = (lax.broadcasted_iota(jnp.int32, (128, 128), 0) // DH
                 == lax.broadcasted_iota(jnp.int32, (128, 128), 1) // DH)

    g_bits = pltpu.bitcast(jnp.broadcast_to(g_w[:, 0:128], (8, 128)), jnp.int32)
    always = (g_bits | 1) != 0

    def matmul(lhs, rhs, dims, side, per_pass):
        m, k = lhs.shape
        cols = [lhs[:, blk(j, 128)] for j in range(k // 128)]
        prev, site, sites = st["prev"], 0, k // 512 * per_pass
        for j in range(0, k // 128, 4):
            groups = [cols[j][blk(i, 16)] for i in range(m // 16)]
            for i in range(0, m // 16, m // 16 // per_pass):
                st["after"] = prev[blk(site * (prev.shape[0] // 8) // sites, 8)]
                site += 1
                v = next(side, None)
                if v is not None:
                    kept = jnp.where(always, pltpu.bitcast(groups[i], jnp.int32), pltpu.bitcast(v, jnp.int32))
                    groups[i] = pltpu.bitcast(kept, BF16)
            cols[j] = jnp.concatenate(groups, axis=0)
        st["prev"] = lax.dot_general(jnp.concatenate(cols, axis=1), rhs, (dims, ((), ())),
                                     preferred_element_type=F32)
        return st["prev"]

    def held(v):
        after = jnp.tile(st["after"], (v.shape[0] // 8, v.shape[1] // 128))
        return jnp.where(jnp.tile(always, (v.shape[0] // 8, v.shape[1] // 128)), v, after)

    NN, NT = ((1,), (0,)), ((1,), (1,))
    st = {"best": jnp.full((16, 1), -jnp.inf, F32), "idx": jnp.zeros((16, 1), jnp.int32),
          "y": [jnp.zeros((8, 128), F32)] * (D // 128),
          "prev": jnp.zeros((8, 128), F32), "after": jnp.zeros((8, 128), F32)}

    def weights_work(b):
        out = []
        for w_v in (wk_v, wq_v):
            cols = []
            for j in range(D // 128):
                w = pltpu.bitcast(held(pltpu.bitcast(w_v[b, blk(j, 128), :], F32)), BF16)
                cols.append(w.T)
                yield pltpu.bitcast(cols[-1][112:128], jnp.int32) | pltpu.bitcast(cols[-1][240:256], jnp.int32)
            out.append(jnp.concatenate(cols, axis=1))
        st["wt"] = jnp.concatenate(out, axis=0)

    def norm_work(b, pq, z):
        zb = jnp.broadcast_to(z, (RK, 128))
        for j in range(S // 128):
            out = []
            zj = held(zb)
            for h in range(RK // DH):
                ph = pq[j][blk(h, DH)].astype(F32)
                den = jnp.sum(ph * zj[blk(h, DH)], axis=0, keepdims=True) + 1e-6
                out.append((ph * (1.0 / den)).astype(BF16))
            out = jnp.concatenate(out, axis=0).T
            pqn_v[blk(j, 128), blk(b, RK)] = out
            last = pltpu.bitcast(out[112:128], jnp.int32)
            yield last[:, 0:128] | last[:, 128:256]

    def route_work():
        g_w8, w_r8 = jnp.broadcast_to(g_w, (8, D)), jnp.broadcast_to(w_r, (8, D))
        for t in range(0, S, 16):
            g = _sigmoid(_rowdot(x_v[t:t + 16, :], held(g_w8)))
            g_v[t:t + 16, :] = jnp.broadcast_to(g, (16, 128))
            r = _rbf(_rowdot(bx_v[t:t + 16, :], held(w_r8)))
            better = r > st["best"]
            st["best"] = jnp.where(better, r, st["best"])
            st["idx"] = jnp.where(better, t, st["idx"])
            both = g + st["best"]
            yield jnp.broadcast_to(both[0:8] + both[8:16], (8, 128))

    def ffn_work():
        for c in range(0, F, 128):
            acc = []
            for w_v in (wg_v, wu_v):
                a = jnp.zeros((8, 128), F32)
                for k in range(D // 16):
                    if k % 16 == 0:
                        a = held(a)
                    pr = w_v[blk(k, 16), c:c + 128].astype(F32) * xcol_v[blk(k, 16), :]
                    a = a + pr[0:8] + pr[8:16]
                    if k % 16 == 15:
                        yield a
                acc.append(_rbf(jnp.sum(a, axis=0, keepdims=True)))
            gate, up = acc
            hcol = _to_col(_rbf(_rbf(gate * _sigmoid(gate)) * up))
            for n in range(D // 128):
                y = held(st["y"][n])
                for k in range(128 // 16):
                    pr = wd_v[c + k * 16:c + (k + 1) * 16, blk(n, 128)].astype(F32) * hcol[blk(k, 16)]
                    y = y + pr[0:8] + pr[8:16]
                st["y"][n] = y
                if n % 2 == 1:
                    yield y + st["y"][n - 1]

    def chain(*gens):
        for gen in gens:
            yield from gen

    def drain(gen):
        for _ in gen:
            pass

    def kq_proj(lo, hi, side, per_pass):
        out = []
        for c in range(lo, hi, 128):
            out.append(_phi(matmul(st["wt"], x_v[c:c + 128, :], NT, side, per_pass)).astype(BF16))
        return out

    def k_step(b, p, side, per_pass):
        pk = [t[0:RK] for t in p]
        zacc = pk[0].astype(F32)
        for t in pk[1:]:
            zacc = zacc + t.astype(F32)
        z = _rbf(jnp.sum(zacc, axis=1, keepdims=True))
        own = norm_work(b, [t[RK:2 * RK] for t in p], z)
        if b + 1 < NK:
            own = chain(weights_work(b + 1), own)
        both = chain(own, side)
        pk = jnp.concatenate(pk, axis=1)
        gm = jnp.concatenate([matmul(pk, x_v[:, blk(n, 128)], NN, both, per_pass).astype(BF16)
                              for n in range(D // 128)], axis=1)
        drain(own)
        for j in range(RK // 128):
            rows = blk(b * (RK // 128) + j, 128)
            kv = jnp.dot(gm[blk(j, 128)], wv_v[b, :, blk(j, 128)], preferred_element_type=F32)
            kv = jnp.where(same_head, kv, 0.0).astype(BF16)
            m_v[rows, :] = jnp.dot(kv, wo_v[rows, :], preferred_element_type=F32).astype(BF16)

    nothing = iter(())
    start(cp_wk[0], cp_wq[0], cp_x[0])
    wait(cp_wk[0], cp_wq[0])
    start(cp_x[1])
    drain(weights_work(0))
    p = []
    for i, (lo, hi) in enumerate(X_CHUNKS):
        if i + 2 < len(X_CHUNKS):
            start(cp_x[i + 2])
        elif i + 2 == len(X_CHUNKS):
            start(cp_wv[0], cp_wo[0], cp_wk[1], cp_wq[1])
        else:
            start(*cp_bx)
        wait(cp_x[i])
        p += kq_proj(lo, hi, nothing, 1)
    start(cp_wv[1], cp_wo[1], cp_wk[2], cp_wq[2])
    wait(cp_wv[0], cp_wo[0], cp_wk[1], cp_wq[1])
    k_step(0, p, nothing, 1)

    start(cp_wv[2], cp_wo[2], cp_wk[3], cp_wq[3], cp_wg[0], cp_wu[0], cp_wd[0])
    wait(cp_wv[1], cp_wo[1], cp_wk[2], cp_wq[2], *cp_bx)
    route = route_work()
    k_step(1, kq_proj(0, S, route, 4), nothing, 1)
    drain(route)
    best = jnp.max(st["best"], axis=0, keepdims=True)
    pos = st["idx"] + lax.broadcasted_iota(jnp.int32, (16, 1), 0)
    idx = jnp.min(jnp.where(st["best"] == best, pos, S - 1), axis=0, keepdims=True)[0, 0]
    idx = jnp.clip(idx, 0, S - 1)
    grp = pl.multiple_of((idx // 16) * 16, 16)
    sel = lax.broadcasted_iota(jnp.int32, (16, 1), 0) == idx - grp

    start(cp_wv[3], cp_wo[3], cp_wg[1], cp_wu[1], cp_wd[1])
    wait(cp_wv[2], cp_wo[2], cp_wk[3], cp_wq[3])
    b_grp = bx_v[pl.ds(grp, 16), :].astype(F32)
    xcol_v[...] = _to_col(jnp.sum(jnp.where(sel, b_grp, 0.0), axis=0, keepdims=True))
    k_step(2, kq_proj(0, S, nothing, 1), nothing, 1)

    wait(cp_wv[3], cp_wo[3], cp_wg[0], cp_wu[0], cp_wd[0])
    ffn = ffn_work()
    first = (next(ffn) for _ in range(F_CHUNKS[0][1] // 128 * 12))
    k_step(3, kq_proj(0, S, first, 4), first, 2)
    drain(first)

    t_sel = idx // TO
    cp_o = [copy(o_v.at[blk(t, TO)], o_hbm.at[blk(t, TO)], s_o.at[t]) for t in range(NO)]
    cp_fix = copy(o_v.at[pl.ds(grp, 16)], o_hbm.at[pl.ds(grp, 16)], s_o.at[NO])
    wait(cp_wg[1], cp_wu[1], cp_wd[1])
    for t in range(NO):
        rows = blk(t, TO)
        slot = (t_sel == t).astype(jnp.int32)
        g = g_v[rows, :]
        for n in range(D // 128):
            a = matmul(pqn_v[rows, :], m_v[:, blk(n, 128)], NN, ffn, 4)
            a_v[slot, :, blk(n, 128)] = a
            bt = bx_v[rows, blk(n, 128)].astype(F32)
            o_v[rows, blk(n, 128)] = (g * a + (1.0 - g) * (bt + bt * 0.0)).astype(BF16)
        if t == NO - 2:
            drain(ffn)
        if t < NO - 1:
            cp_o[t].start()

    y = _rbf(_rbf(jnp.sum(jnp.concatenate(st["y"], axis=1), axis=0, keepdims=True)) * _rbf(_sigmoid(best)))
    g = jnp.tile(g_v[pl.ds(grp, 16), :], (1, D // 128))
    a = a_v[1, pl.ds(pl.multiple_of(grp - t_sel * TO, 16), 16), :]
    b_new = b_grp + (b_grp * 0.0 + jnp.where(sel, y, 0.0))
    wait(*cp_o[:NO - 1])
    o_v[pl.ds(grp, 16), :] = (g * a + (1.0 - g) * b_new).astype(BF16)
    cp_o[NO - 1].start()

    @pl.when(t_sel < NO - 1)
    def _():
        cp_fix.start()
        cp_fix.wait()

    cp_o[NO - 1].wait()


@jax.jit
def pallas_gated_mix__linear_attn_block__moe_arch_mod__prompt_kernel(
    A_x: jax.Array,
    A_wqkv: jax.Array,
    A_wo: jax.Array,
    B_x: jax.Array,
    B_w_r: jax.Array,
    B_w_gate: jax.Array,
    B_w_up: jax.Array,
    B_w_down: jax.Array,
    gate_w: jax.Array,
):
    hbm = pl.BlockSpec(memory_space=pl.ANY)
    vmem = pl.BlockSpec(memory_space=pltpu.VMEM)
    dma = pltpu.SemaphoreType.DMA
    out = pl.pallas_call(
        _kernel,
        out_shape=jax.ShapeDtypeStruct((S, D), BF16),
        in_specs=[hbm, hbm, hbm, hbm, vmem, hbm, hbm, hbm, vmem],
        out_specs=hbm,
        scratch_shapes=[
            pltpu.VMEM((S, D), BF16),
            pltpu.VMEM((S, D), BF16),
            pltpu.VMEM((NK, D, RK), BF16),
            pltpu.VMEM((NK, D, RK), BF16),
            pltpu.VMEM((NK, D, RK), BF16),
            pltpu.VMEM((D, D), BF16),
            pltpu.VMEM((D, F), BF16),
            pltpu.VMEM((D, F), BF16),
            pltpu.VMEM((F, D), BF16),
            pltpu.VMEM((S, D), BF16),
            pltpu.VMEM((D, D), BF16),
            pltpu.VMEM((S, 128), F32),
            pltpu.VMEM((D, 128), F32),
            pltpu.VMEM((S, D), BF16),
            pltpu.VMEM((2, TO, D), F32),
            dma((len(X_CHUNKS),)), dma((NO,)), dma((NK,)), dma((NK,)), dma((NK,)), dma((NK,)),
            dma((NF,)), dma((NF,)), dma((NF,)), dma((NO + 1,)),
        ],
        compiler_params=pltpu.CompilerParams(vmem_limit_bytes=100 * 1024 * 1024),
    )(A_x.reshape(S, D), A_wqkv, A_wo, B_x.reshape(S, D), B_w_r,
      B_w_gate, B_w_up, B_w_down, gate_w)
    return out.reshape(1, S, D)
```

```python
import jax
import jax.numpy as jnp
from jax import lax
import jax.experimental.pallas as pl
import jax.experimental.pallas.tpu as pltpu

S, D, F, H = 2048, 1024, 3584, 32
DH = D // H
RK = 256
TO = 512
NK, NO = D // RK, S // TO
F_CHUNKS = ((0, 1408), (1408, 2816), (2816, 3584))
NF = len(F_CHUNKS)
X_CHUNKS = ((0, 256), (256, 512), (512, 1024), (1024, 2048))
F32, BF16 = jnp.float32, jnp.bfloat16


def _phi(t):
    return jnp.where(t > 0, t + 1.0, jnp.exp(t)) + 1e-6


def _sigmoid(t):
    return 1.0 / (1.0 + jnp.exp(-t))


def _rbf(t):
    return t.astype(BF16).astype(F32)


def _rowdot(a, w, first):
    acc = None
    for j in range(0, D, 128):
        wj = first(w[:, 0:128]) if j == 0 else w[:, j:j + 128]
        pr = a[:, j:j + 128].astype(F32) * jnp.concatenate([wj, wj], axis=0)
        acc = pr if j == 0 else acc + pr
    return jnp.sum(acc, axis=1, keepdims=True)


def _to_col(row):
    return jnp.broadcast_to(row, (128, row.shape[1])).T


def _kernel(x_hbm, wqkv_hbm, wo_hbm, bx_hbm, wr_ref, wg_hbm, wu_hbm, wd_hbm, gw_ref,
            o_hbm,
            x_v, bx_v, wq_v, wk_v, wv_v, wo_v, wg_v, wu_v, wd_v,
            pqn_v, m_v, g_v, xcol_v, o_v, a_v,
            s_x, s_bx, s_wq, s_wk, s_wv, s_wo, s_wg, s_wu, s_wd, s_o):
    copy = pltpu.make_async_copy

    def blk(i, n):
        return slice(i * n, (i + 1) * n)

    cp_x = [copy(x_hbm.at[lo:hi], x_v.at[lo:hi], s_x.at[i]) for i, (lo, hi) in enumerate(X_CHUNKS)]
    cp_bx = [copy(bx_hbm.at[blk(t, TO)], bx_v.at[blk(t, TO)], s_bx.at[t]) for t in range(NO)]
    cp_wq = [copy(wqkv_hbm.at[:, blk(b, RK)], wq_v.at[b], s_wq.at[b]) for b in range(NK)]
    cp_wk = [copy(wqkv_hbm.at[:, blk(NK + b, RK)], wk_v.at[b], s_wk.at[b]) for b in range(NK)]
    cp_wv = [copy(wqkv_hbm.at[:, blk(2 * NK + b, RK)], wv_v.at[b], s_wv.at[b]) for b in range(NK)]
    cp_wo = [copy(wo_hbm.at[blk(b, RK)], wo_v.at[blk(b, RK)], s_wo.at[b]) for b in range(NK)]
    cp_wg = [copy(wg_hbm.at[:, lo:hi], wg_v.at[:, lo:hi], s_wg.at[c]) for c, (lo, hi) in enumerate(F_CHUNKS)]
    cp_wu = [copy(wu_hbm.at[:, lo:hi], wu_v.at[:, lo:hi], s_wu.at[c]) for c, (lo, hi) in enumerate(F_CHUNKS)]
    cp_wd = [copy(wd_hbm.at[lo:hi], wd_v.at[lo:hi], s_wd.at[c]) for c, (lo, hi) in enumerate(F_CHUNKS)]

    def start(*cps):
        for c in cps:
            c.start()

    def wait(*cps):
        for c in cps:
            c.wait()

    w_r = wr_ref[...].astype(F32).reshape(1, D)
    g_w = gw_ref[...].astype(F32).reshape(1, D)
    same_head = (lax.broadcasted_iota(jnp.int32, (128, 128), 0) // DH
                 == lax.broadcasted_iota(jnp.int32, (128, 128), 1) // DH)

    g_bits = pltpu.bitcast(jnp.broadcast_to(g_w[:, 0:128], (8, 128)), jnp.int32)
    always = (g_bits | 1) != 0

    st = {"best": jnp.full((16, 1), -jnp.inf, F32), "idx": jnp.zeros((16, 1), jnp.int32),
          "y": [jnp.zeros((8, 128), F32)] * (D // 128),
          "prev": [jnp.zeros((8, 128), F32)] * 2, "after": jnp.zeros((8, 128), F32)}

    def bits(v):
        return pltpu.bitcast(v, jnp.int32)

    def matmul(lhs, rhs, side, rhs_t=False, acc=None):
        m, k = lhs.shape
        site = 0
        for c in range(0, k, 512):
            first = [lhs[blk(i, 16), c:c + 128] for i in range(m // 16)]
            for i in range(0, m // 16, 8):
                prev = st["prev"][-(512 // m)]
                st["after"] = prev[blk(i * 16 * prev.shape[0] // m // 8, 8)]
                vals = [next(gen, None) for gen, stride in side if site % stride == 0]
                site += 1
                for v in vals:
                    if v is not None:
                        first[i] = pltpu.bitcast(jnp.where(always, bits(first[i]), bits(v)), BF16)
            a = jnp.concatenate([jnp.concatenate(first, axis=0), lhs[:, c + 128:c + 512]], axis=1)
            if rhs_t:
                part = lax.dot_general(a, rhs[:, c:c + 512], (((1,), (1,)), ((), ())),
                                       preferred_element_type=F32)
            else:
                part = jnp.dot(a, rhs[c:c + 512, :], preferred_element_type=F32)
            st["prev"].append(part)
            acc = part if acc is None else acc + part
        return acc

    def held(v):
        reps = (v.shape[0] // 8, v.shape[1] // 128)
        return jnp.where(jnp.tile(always, reps), v, jnp.tile(st["after"], reps))

    def transpose_work(name, w_v, b):
        cols = []
        for j in range(D // 128):
            cols.append(pltpu.bitcast(held(pltpu.bitcast(w_v[b, blk(j, 128), :], F32)), BF16).T)
            if j == D // 128 - 1:
                st[name] = jnp.concatenate(cols, axis=1)
            yield bits(cols[-1][112:128]) | bits(cols[-1][240:256])

    def norm_work(b, pq, z):
        zb = jnp.broadcast_to(z, (RK, 128))
        heads = range(RK // DH)
        for j in range(S // 128):
            ph = [pq[j][blk(h, DH)].astype(F32) for h in heads]
            den = [jnp.sum(ph[h] * zb[blk(h, DH)], axis=0, keepdims=True) for h in heads]
            inv = 1.0 / (held(jnp.concatenate(den, axis=0)) + 1e-6)
            yield inv
            inv = held(inv)
            out = jnp.concatenate([(ph[h] * inv[h:h + 1]).astype(BF16) for h in heads], axis=0).T
            pqn_v[blk(j, 128), blk(b, RK)] = out
            yield bits(out[112:128, 0:128]) | bits(out[112:128, 128:256])

    def route_work():
        g_w8, w_r8 = jnp.broadcast_to(g_w, (8, D)), jnp.broadcast_to(w_r, (8, D))
        for t in range(0, S, 16):
            g = _sigmoid(_rowdot(x_v[t:t + 16, :], g_w8, held))
            g_v[t:t + 16, :] = jnp.broadcast_to(g, (16, 128))
            r = _rbf(_rowdot(bx_v[t:t + 16, :], w_r8, held))
            better = r > st["best"]
            st["best"] = jnp.where(better, r, st["best"])
            st["idx"] = jnp.where(better, t, st["idx"])
            both = g + st["best"]
            yield jnp.broadcast_to(both[0:8] + both[8:16], (8, 128))

    def select_work():
        best = jnp.max(st["best"], axis=0, keepdims=True)
        pos = st["idx"] + lax.broadcasted_iota(jnp.int32, (16, 1), 0)
        idx = jnp.min(jnp.where(st["best"] == best, pos, S - 1), axis=0, keepdims=True)[0, 0]
        idx = jnp.clip(idx, 0, S - 1)
        grp = pl.multiple_of((idx // 16) * 16, 16)
        sel = lax.broadcasted_iota(jnp.int32, (16, 1), 0) == idx - grp
        b_grp = bx_v[pl.ds(grp, 16), :].astype(F32)
        xcol = _to_col(jnp.sum(jnp.where(sel, b_grp, 0.0), axis=0, keepdims=True))
        xcol_v[...] = xcol
        st.update(score=best, tok=idx, grp=grp, sel=sel, b_grp=b_grp)
        yield xcol[D - 8:D]

    def ffn_work():
        for c in range(0, F, 128):
            acc = []
            for w_v in (wg_v, wu_v):
                a = jnp.zeros((8, 128), F32)
                for k in range(D // 16):
                    if k % 16 == 0:
                        a = held(a)
                    pr = w_v[blk(k, 16), c:c + 128].astype(F32) * xcol_v[blk(k, 16), :]
                    a = a + pr[0:8] + pr[8:16]
                    if k % 16 == 15:
                        yield a
                acc.append(_rbf(jnp.sum(a, axis=0, keepdims=True)))
            gate, up = acc
            hcol = _to_col(_rbf(_rbf(gate * _sigmoid(gate)) * up))
            for n in range(D // 128):
                y = held(st["y"][n])
                for k in range(128 // 16):
                    pr = wd_v[c + k * 16:c + (k + 1) * 16, blk(n, 128)].astype(F32) * hcol[blk(k, 16)]
                    y = y + pr[0:8] + pr[8:16]
                st["y"][n] = y
                if n % 2 == 1:
                    yield y + st["y"][n - 1]

    def drain(gen):
        for _ in gen:
            pass

    def mix_work(b, gm):
        kv = []
        for i in range(RK // 128):
            t = jnp.dot(gm[blk(i, 128)], wv_v[b, :, blk(i, 128)], preferred_element_type=F32)
            kv.append(jnp.where(same_head, t, 0.0).astype(BF16))
        yield
        for i in range(RK // 128):
            rows = blk(b * (RK // 128) + i, 128)
            m_v[rows, :] = jnp.dot(kv[i], wo_v[rows, :], preferred_element_type=F32).astype(BF16)
        yield

    def k_step(b, mix, side, g_side, arrive=None):
        wt = jnp.concatenate([st["wk"], st["wq"]], axis=0)
        pk, pq, zacc = [], [], None
        for j in range(S // 128):
            if arrive is not None:
                arrive(j)
            p = _phi(matmul(wt, x_v[blk(j, 128), :], side, rhs_t=True)).astype(BF16)
            pk.append(p[0:RK])
            pq.append(p[RK:2 * RK])
            zacc = pk[j].astype(F32) if j == 0 else zacc + pk[j].astype(F32)
            next(mix, None)
        z = _rbf(jnp.sum(zacc, axis=1, keepdims=True))
        pk = jnp.concatenate(pk, axis=1)
        if arrive is not None:
            arrive(S // 128)
        own = [transpose_work(n, w, b + 1) for n, w in (("wk", wk_v), ("wq", wq_v)) if b + 1 < NK]
        norm = norm_work(b, pq, z)
        gm = [matmul(pk, x_v[:, blk(n, 128)],
                     [(norm, 2)] + [(w, 2) for w in own[n // 4:n // 4 + 1]] + g_side).astype(BF16)
              for n in range(D // 128)]
        for gen in own + [norm]:
            drain(gen)
        return mix_work(b, jnp.concatenate(gm, axis=1))

    later = [[cp_x[2]], [cp_x[3]], [cp_wk[1], cp_wq[1]], [cp_wv[0], cp_wo[0], *cp_bx]]

    def arrive(j):
        for i, (lo, _) in enumerate(X_CHUNKS):
            if lo == j * 128:
                start(*later[i])
                wait(cp_x[i])
        if j == S // 128:
            start(cp_wk[2], cp_wq[2], cp_wv[1], cp_wo[1])
            wait(cp_wk[1], cp_wq[1])

    start(cp_wk[0], cp_wq[0], cp_x[0])
    wait(cp_wk[0], cp_wq[0])
    start(cp_x[1])
    drain(transpose_work("wk", wk_v, 0))
    drain(transpose_work("wq", wq_v, 0))
    mix = k_step(0, iter(()), [], [], arrive)

    start(cp_wk[3], cp_wq[3], cp_wv[2], cp_wo[2], cp_wg[0], cp_wu[0], cp_wd[0])
    wait(cp_wv[0], cp_wo[0], *cp_bx, cp_wk[2], cp_wq[2])
    mix = k_step(1, mix, [(route_work(), 1)], [(select_work(), 1)])

    start(cp_wv[3], cp_wo[3], cp_wg[1], cp_wu[1], cp_wd[1])
    wait(cp_wv[1], cp_wo[1], cp_wk[3], cp_wq[3], cp_wg[0], cp_wu[0], cp_wd[0])
    ffn = ffn_work()
    mix = k_step(2, mix, [(ffn, 1)], [])

    start(cp_wg[2], cp_wu[2], cp_wd[2])
    wait(cp_wv[2], cp_wo[2], cp_wv[3], cp_wo[3], cp_wg[1], cp_wu[1], cp_wd[1])
    mix = k_step(3, mix, [(ffn, 1)], [])

    grp, sel, b_grp = st["grp"], st["sel"], st["b_grp"]
    t_sel = st["tok"] // TO
    cp_o = [copy(o_v.at[blk(t, TO)], o_hbm.at[blk(t, TO)], s_o.at[t]) for t in range(NO)]
    cp_fix = copy(o_v.at[pl.ds(grp, 16)], o_hbm.at[pl.ds(grp, 16)], s_o.at[NO])
    wait(cp_wg[2], cp_wu[2], cp_wd[2])
    for t in range(NO):
        rows = blk(t, TO)
        slot = (t_sel == t).astype(jnp.int32)
        g = g_v[rows, :]
        half = {}
        if t == 0:
            for n in range(4):
                half[n] = matmul(pqn_v[rows, 0:512], m_v[0:512, blk(n, 128)], [(ffn, 1)])
                next(mix, None)
        for n in range(D // 128):
            if n in half:
                a = matmul(pqn_v[rows, 512:D], m_v[512:D, blk(n, 128)], [(ffn, 1)], acc=half[n])
            else:
                a = matmul(pqn_v[rows, :], m_v[:, blk(n, 128)], [(ffn, 1)])
            a_v[slot, :, blk(n, 128)] = a
            bt = bx_v[rows, blk(n, 128)].astype(F32)
            o_v[rows, blk(n, 128)] = (g * a + (1.0 - g) * (bt + bt * 0.0)).astype(BF16)
        if t == NO - 2:
            drain(ffn)
        if t < NO - 1:
            cp_o[t].start()

    y = _rbf(_rbf(jnp.sum(jnp.concatenate(st["y"], axis=1), axis=0, keepdims=True)) * _rbf(_sigmoid(st["score"])))
    g = jnp.tile(g_v[pl.ds(grp, 16), :], (1, D // 128))
    a = a_v[1, pl.ds(pl.multiple_of(grp - t_sel * TO, 16), 16), :]
    b_new = b_grp + (b_grp * 0.0 + jnp.where(sel, y, 0.0))
    wait(*cp_o[:NO - 1])
    o_v[pl.ds(grp, 16), :] = (g * a + (1.0 - g) * b_new).astype(BF16)
    cp_o[NO - 1].start()

    @pl.when(t_sel < NO - 1)
    def _():
        cp_fix.start()
        cp_fix.wait()

    cp_o[NO - 1].wait()


@jax.jit
def pallas_gated_mix__linear_attn_block__moe_arch_mod__prompt_kernel(
    A_x: jax.Array,
    A_wqkv: jax.Array,
    A_wo: jax.Array,
    B_x: jax.Array,
    B_w_r: jax.Array,
    B_w_gate: jax.Array,
    B_w_up: jax.Array,
    B_w_down: jax.Array,
    gate_w: jax.Array,
):
    hbm = pl.BlockSpec(memory_space=pl.ANY)
    vmem = pl.BlockSpec(memory_space=pltpu.VMEM)
    dma = pltpu.SemaphoreType.DMA
    out = pl.pallas_call(
        _kernel,
        out_shape=jax.ShapeDtypeStruct((S, D), BF16),
        in_specs=[hbm, hbm, hbm, hbm, vmem, hbm, hbm, hbm, vmem],
        out_specs=hbm,
        scratch_shapes=[
            pltpu.VMEM((S, D), BF16),
            pltpu.VMEM((S, D), BF16),
            pltpu.VMEM((NK, D, RK), BF16),
            pltpu.VMEM((NK, D, RK), BF16),
            pltpu.VMEM((NK, D, RK), BF16),
            pltpu.VMEM((D, D), BF16),
            pltpu.VMEM((D, F), BF16),
            pltpu.VMEM((D, F), BF16),
            pltpu.VMEM((F, D), BF16),
            pltpu.VMEM((S, D), BF16),
            pltpu.VMEM((D, D), BF16),
            pltpu.VMEM((S, 128), F32),
            pltpu.VMEM((D, 128), F32),
            pltpu.VMEM((S, D), BF16),
            pltpu.VMEM((2, TO, D), F32),
            dma((len(X_CHUNKS),)), dma((NO,)), dma((NK,)), dma((NK,)), dma((NK,)), dma((NK,)),
            dma((NF,)), dma((NF,)), dma((NF,)), dma((NO + 1,)),
        ],
        compiler_params=pltpu.CompilerParams(vmem_limit_bytes=100 * 1024 * 1024),
    )(A_x.reshape(S, D), A_wqkv, A_wo, B_x.reshape(S, D), B_w_r,
      B_w_gate, B_w_up, B_w_down, gate_w)
    return out.reshape(1, S, D)
```

```python
import jax
import jax.numpy as jnp
from jax import lax
import jax.experimental.pallas as pl
import jax.experimental.pallas.tpu as pltpu

S, D, F, H = 2048, 1024, 3584, 32
DH = D // H
RK = 256
TO = 512
NK, NO = D // RK, S // TO
F_CHUNKS = ((0, 768), (768, 1536), (1536, 2944), (2944, 3584))
NF = len(F_CHUNKS)
X_CHUNKS = ((0, 256), (256, 640), (640, 1280), (1280, 2048))
O_STRIPS = (3, 5, 7, 8)
N_GROUPS, EARLY = 12, 5
F32, BF16 = jnp.float32, jnp.bfloat16


def _phi(t):
    return jnp.where(t > 0, t + 1.0, jnp.exp(t)) + 1e-6


def _sigmoid(t):
    return 1.0 / (1.0 + jnp.exp(-t))


def _rbf(t):
    return t.astype(BF16).astype(F32)


def _rowdot(a, w, first):
    acc = None
    for j in range(0, D, 128):
        wj = first(w[:, 0:128]) if j == 0 else w[:, j:j + 128]
        pr = a[:, j:j + 128].astype(F32) * jnp.concatenate([wj, wj], axis=0)
        acc = pr if j == 0 else acc + pr
    return jnp.sum(acc, axis=1, keepdims=True)


def _to_col(row):
    return jnp.broadcast_to(row, (128, row.shape[1])).T


def _kernel(x_hbm, wqkv_hbm, wo_hbm, bx_hbm, wr_hbm, wg_hbm, wu_hbm, wd_hbm, gw_hbm,
            o_hbm,
            wr_v, gw_v, pilot_v, x_v, bx_v, wq_v, wk_v, wv_v, wo_v, wg_v, wu_v, wd_v,
            pqn_v, m_v, g_v, xcol_v, o_v,
            sems):
    copy = pltpu.make_async_copy

    def blk(i, n):
        return slice(i * n, (i + 1) * n)

    x_ = [(x_hbm.at[lo:hi], x_v.at[lo:hi]) for lo, hi in X_CHUNKS]
    kq_ = [[(wqkv_hbm.at[:, blk(NK + b, RK)], wk_v.at[b]), (wqkv_hbm.at[:, blk(b, RK)], wq_v.at[b])]
           for b in range(NK)]
    vo_ = [[(wqkv_hbm.at[:, blk(2 * NK + b, RK)], wv_v.at[b]),
            (wo_hbm.at[blk(b, RK)], wo_v.at[blk(b, RK)])] for b in range(NK)]
    ffn_ = [[(wg_hbm.at[:, lo:hi], wg_v.at[:, lo:hi]), (wu_hbm.at[:, lo:hi], wu_v.at[:, lo:hi]),
             (wd_hbm.at[lo:hi], wd_v.at[lo:hi])] for lo, hi in F_CHUNKS]
    groups = [[(gw_hbm, gw_v), (wr_hbm, wr_v)], kq_[0][:1], kq_[0][1:], x_[0:1], x_[1:2], x_[2:3],
              kq_[1] + x_[3:4], vo_[0] + [(bx_hbm, bx_v)] + kq_[2], ffn_[0], kq_[3] + vo_[1] + ffn_[1],
              vo_[2] + ffn_[2], vo_[3] + ffn_[3]]

    def pilot(i):
        return copy(wo_hbm.at[0:16, 0:128], pilot_v.at[i - EARLY], sems.at[i])

    def start(i):
        if EARLY <= i + 1 < len(groups):
            pilot(i + 1).start()
        for src, dst in groups[i]:
            copy(src, dst, sems.at[i]).start()
        if i >= EARLY:
            pilot(i).wait()

    def wait(i):
        for src, dst in groups[i]:
            copy(src, dst, sems.at[i]).wait()

    for i in range(EARLY):
        start(i)
    wait(0)
    w_r = wr_v[...].astype(F32).reshape(1, D)
    g_w = gw_v[...].astype(F32).reshape(1, D)
    g_bits = pltpu.bitcast(jnp.broadcast_to(g_w[:, 0:128], (8, 128)), jnp.int32)
    always = (g_bits | 1) != 0
    same_head = (lax.broadcasted_iota(jnp.int32, (128, 128), 0) // DH
                 == lax.broadcasted_iota(jnp.int32, (128, 128), 1) // DH)

    st = {"best": jnp.full((16, 1), -jnp.inf, F32), "idx": jnp.zeros((16, 1), jnp.int32),
          "y": [jnp.zeros((8, 128), F32)] * (D // 128),
          "prev": [jnp.zeros((8, 128), F32)] * 2, "after": jnp.zeros((8, 128), F32)}

    def bits(v):
        return pltpu.bitcast(v, jnp.int32)

    def matmul(lhs, rhs, side, rhs_t=False, acc=None):
        m, k = lhs.shape
        site = 0
        for c in range(0, k, 512):
            first = [lhs[blk(i, 16), c:c + 128] for i in range(m // 16)]
            for i in range(0, m // 16, 8):
                prev = st["prev"][-(512 // m)]
                st["after"] = prev[blk(i * 16 * prev.shape[0] // m // 8, 8)]
                vals = [next(gen, None) for gen, stride in side if site % stride == 0]
                site += 1
                for v in vals:
                    if v is not None:
                        first[i] = pltpu.bitcast(jnp.where(always, bits(first[i]), bits(v)), BF16)
            a = jnp.concatenate([jnp.concatenate(first, axis=0), lhs[:, c + 128:c + 512]], axis=1)
            if rhs_t:
                part = lax.dot_general(a, rhs[:, c:c + 512], (((1,), (1,)), ((), ())),
                                       preferred_element_type=F32)
            else:
                part = jnp.dot(a, rhs[c:c + 512, :], preferred_element_type=F32)
            st["prev"].append(part)
            acc = part if acc is None else acc + part
        return acc

    def held(v):
        reps = (v.shape[0] // 8, v.shape[1] // 128)
        return jnp.where(jnp.tile(always, reps), v, jnp.tile(st["after"], reps))

    def transpose_work(name, w_v, b):
        cols = []
        for j in range(D // 128):
            cols.append(pltpu.bitcast(held(pltpu.bitcast(w_v[b, blk(j, 128), :], F32)), BF16).T)
            if j == D // 128 - 1:
                st[name] = jnp.concatenate(cols, axis=1)
            yield bits(cols[-1][112:128]) | bits(cols[-1][240:256])

    def norm_work(b, pq, z):
        zb = jnp.broadcast_to(z, (RK, 128))
        heads = range(RK // DH)
        for j in range(S // 128):
            ph = [pq[j][blk(h, DH)].astype(F32) for h in heads]
            den = [jnp.sum(ph[h] * zb[blk(h, DH)], axis=0, keepdims=True) for h in heads]
            inv = 1.0 / (held(jnp.concatenate(den, axis=0)) + 1e-6)
            yield inv
            inv = held(inv)
            out = jnp.concatenate([(ph[h] * inv[h:h + 1]).astype(BF16) for h in heads], axis=0).T
            pqn_v[blk(j, 128), blk(b, RK)] = out
            yield bits(out[112:128, 0:128]) | bits(out[112:128, 128:256])

    def route_work():
        g_w8, w_r8 = jnp.broadcast_to(g_w, (8, D)), jnp.broadcast_to(w_r, (8, D))
        for t in range(0, S, 16):
            g = _sigmoid(_rowdot(x_v[t:t + 16, :], g_w8, held))
            g_v[t:t + 16, :] = jnp.broadcast_to(g, (16, 128))
            r = _rbf(_rowdot(bx_v[t:t + 16, :], w_r8, held))
            better = r > st["best"]
            st["best"] = jnp.where(better, r, st["best"])
            st["idx"] = jnp.where(better, t, st["idx"])
            both = g + st["best"]
            yield jnp.broadcast_to(both[0:8] + both[8:16], (8, 128))

    def select_work():
        best = jnp.max(st["best"], axis=0, keepdims=True)
        pos = st["idx"] + lax.broadcasted_iota(jnp.int32, (16, 1), 0)
        idx = jnp.min(jnp.where(st["best"] == best, pos, S - 1), axis=0, keepdims=True)[0, 0]
        idx = jnp.clip(idx, 0, S - 1)
        grp = pl.multiple_of((idx // 16) * 16, 16)
        sel = lax.broadcasted_iota(jnp.int32, (16, 1), 0) == idx - grp
        b_grp = bx_v[pl.ds(grp, 16), :].astype(F32)
        xcol = _to_col(jnp.sum(jnp.where(sel, b_grp, 0.0), axis=0, keepdims=True))
        xcol_v[...] = xcol
        st.update(score=best, tok=idx)
        yield xcol[D - 8:D]

    def ffn_work(lo, hi):
        for c in range(lo, hi, 128):
            acc = []
            for w_v in (wg_v, wu_v):
                a = jnp.zeros((8, 128), F32)
                for k in range(D // 16):
                    if k in (0, 22, 43):
                        a = held(a)
                    pr = w_v[blk(k, 16), c:c + 128].astype(F32) * xcol_v[blk(k, 16), :]
                    a = a + pr[0:8] + pr[8:16]
                    if k in (21, 42, 63):
                        yield a
                acc.append(_rbf(jnp.sum(a, axis=0, keepdims=True)))
            gate, up = acc
            hcol = _to_col(_rbf(_rbf(gate * _sigmoid(gate)) * up))
            for n in range(D // 128):
                y = held(st["y"][n])
                for k in range(128 // 16):
                    pr = wd_v[c + k * 16:c + (k + 1) * 16, blk(n, 128)].astype(F32) * hcol[blk(k, 16)]
                    y = y + pr[0:8] + pr[8:16]
                st["y"][n] = y
                if n in (2, 5):
                    yield y + st["y"][n - 1] + st["y"][n - 2]
                if n == 7:
                    yield y + st["y"][n - 1]

    def drain(gen):
        for _ in gen:
            pass

    def mix_work(b, gm):
        kv = []
        for i in range(RK // 128):
            t = jnp.dot(gm[blk(i, 128)], wv_v[b, :, blk(i, 128)], preferred_element_type=F32)
            kv.append(jnp.where(same_head, t, 0.0).astype(BF16))
        yield
        for i in range(RK // 128):
            rows = blk(b * (RK // 128) + i, 128)
            m_v[rows, :] = jnp.dot(kv[i], wo_v[rows, :], preferred_element_type=F32).astype(BF16)
        yield

    def k_step(b, mix, side, g_side, arrive=None):
        wt = jnp.concatenate([st["wk"], st["wq"]], axis=0)
        pk, pq, zacc = [], [], None
        for j in range(S // 128):
            if arrive is not None:
                arrive(j)
            p = _phi(matmul(wt, x_v[blk(j, 128), :], side, rhs_t=True)).astype(BF16)
            pk.append(p[0:RK])
            pq.append(p[RK:2 * RK])
            zacc = pk[j].astype(F32) if j == 0 else zacc + pk[j].astype(F32)
            next(mix, None)
        z = _rbf(jnp.sum(zacc, axis=1, keepdims=True))
        pk = jnp.concatenate(pk, axis=1)
        if arrive is not None:
            arrive(S // 128)
        own = [transpose_work(n, w, b + 1) for n, w in (("wk", wk_v), ("wq", wq_v)) if b + 1 < NK]
        norm = norm_work(b, pq, z)
        gm = [matmul(pk, x_v[:, blk(n, 128)],
                     [(norm, 2)] + [(w, 2) for w in own[n // 4:n // 4 + 1]] + g_side).astype(BF16)
              for n in range(D // 128)]
        for gen in own + [norm]:
            drain(gen)
        return mix_work(b, jnp.concatenate(gm, axis=1))

    def arrive(j):
        for i, (lo, _) in enumerate(X_CHUNKS):
            if lo == j * 128:
                start(EARLY + i)
                wait(3 + i)

    wait(1)
    st["wk"] = wk_v[0].T
    wait(2)
    st["wq"] = wq_v[0].T
    mix = k_step(0, iter(()), [], [], arrive)

    start(9)
    wait(7)
    mix = k_step(1, mix, [(route_work(), 1)], [(select_work(), 1)])

    start(10)
    wait(8)
    wait(9)
    ffn = ffn_work(F_CHUNKS[0][0], F_CHUNKS[1][1])
    mix = k_step(2, mix, [(ffn, 1)], [])
    drain(ffn)

    def arrive_last(j):
        if j == S // 128:
            drain(ffn)
            wait(11)

    start(11)
    wait(10)
    ffn, ffn_last = ffn_work(*F_CHUNKS[2]), ffn_work(*F_CHUNKS[3])
    mix = k_step(3, mix, [(ffn, 1)], [(ffn_last, 1)], arrive_last)
    drain(ffn_last)

    y = _rbf(jnp.sum(jnp.concatenate(st["y"], axis=1), axis=0, keepdims=True))
    y = _rbf(y * _rbf(_sigmoid(st["score"])))
    cp_o = []
    for t in range(NO):
        rows = blk(t, TO)
        g = g_v[rows, :]
        routed = lax.broadcasted_iota(jnp.int32, (TO, 128), 0) == st["tok"] - t * TO
        half = {}
        if t == 0:
            for n in range(4):
                half[n] = matmul(pqn_v[rows, 0:512], m_v[0:512, blk(n, 128)], [])
                next(mix, None)
        for n in range(D // 128):
            if n in half:
                a = matmul(pqn_v[rows, 512:D], m_v[512:D, blk(n, 128)], [], acc=half[n])
            else:
                a = matmul(pqn_v[rows, :], m_v[:, blk(n, 128)], [])
            bt = bx_v[rows, blk(n, 128)].astype(F32)
            bt = bt + (bt * 0.0 + jnp.where(routed, y[:, blk(n, 128)], 0.0))
            o_v[rows, blk(n, 128)] = (g * a + (1.0 - g) * bt).astype(BF16)
            if n + 1 in (O_STRIPS if t == NO - 1 else O_STRIPS[-1:]):
                lo = 0 if t < NO - 1 else ((0,) + O_STRIPS)[O_STRIPS.index(n + 1)]
                cols = slice(lo * 128, (n + 1) * 128)
                cp_o.append(copy(o_v.at[rows, cols], o_hbm.at[rows, cols], sems.at[len(groups) + len(cp_o)]))
                cp_o[-1].start()
    for c in cp_o:
        c.wait()


@jax.jit
def pallas_gated_mix__linear_attn_block__moe_arch_mod__prompt_kernel(
    A_x: jax.Array,
    A_wqkv: jax.Array,
    A_wo: jax.Array,
    B_x: jax.Array,
    B_w_r: jax.Array,
    B_w_gate: jax.Array,
    B_w_up: jax.Array,
    B_w_down: jax.Array,
    gate_w: jax.Array,
):
    hbm = pl.BlockSpec(memory_space=pl.ANY)
    out = pl.pallas_call(
        _kernel,
        out_shape=jax.ShapeDtypeStruct((S, D), BF16),
        in_specs=[hbm] * 9,
        out_specs=hbm,
        scratch_shapes=[
            pltpu.VMEM((D,), BF16),
            pltpu.VMEM((D,), BF16),
            pltpu.VMEM((N_GROUPS - EARLY, 16, 128), BF16),
            pltpu.VMEM((S, D), BF16),
            pltpu.VMEM((S, D), BF16),
            pltpu.VMEM((NK, D, RK), BF16),
            pltpu.VMEM((NK, D, RK), BF16),
            pltpu.VMEM((NK, D, RK), BF16),
            pltpu.VMEM((D, D), BF16),
            pltpu.VMEM((D, F), BF16),
            pltpu.VMEM((D, F), BF16),
            pltpu.VMEM((F, D), BF16),
            pltpu.VMEM((S, D), BF16),
            pltpu.VMEM((D, D), BF16),
            pltpu.VMEM((S, 128), F32),
            pltpu.VMEM((D, 128), F32),
            pltpu.VMEM((S, D), BF16),
            pltpu.SemaphoreType.DMA((N_GROUPS + NO - 1 + len(O_STRIPS),)),
        ],
        compiler_params=pltpu.CompilerParams(vmem_limit_bytes=100 * 1024 * 1024),
    )(A_x.reshape(S, D), A_wqkv, A_wo, B_x.reshape(S, D), B_w_r,
      B_w_gate, B_w_up, B_w_down, gate_w)
    return out.reshape(1, S, D)
```

```python
import jax
import jax.numpy as jnp
from jax import lax
import jax.experimental.pallas as pl
import jax.experimental.pallas.tpu as pltpu

S, D, F, H = 2048, 1024, 3584, 32
DH = D // H
RK = 256
TO = 512
NK, NO = D // RK, S // TO
F_CHUNKS = ((0, 768), (768, 1536), (1536, 2944), (2944, 3584))
NF = len(F_CHUNKS)
X_CHUNKS = ((0, 256), (256, 640), (640, 1280), (1280, 2048))
O_STRIPS = (3, 5, 7, 8)
N_GROUPS = 12
F32, BF16 = jnp.float32, jnp.bfloat16


def _phi(t):
    return jnp.where(t > 0, t + 1.0, jnp.exp(t)) + 1e-6


def _sigmoid(t):
    return 1.0 / (1.0 + jnp.exp(-t))


def _rbf(t):
    return t.astype(BF16).astype(F32)


def _rowdot(a, w, first):
    acc = None
    for j in range(0, D, 128):
        wj = first(w[:, 0:128]) if j == 0 else w[:, j:j + 128]
        pr = a[:, j:j + 128].astype(F32) * jnp.concatenate([wj, wj], axis=0)
        acc = pr if j == 0 else acc + pr
    return jnp.sum(acc, axis=1, keepdims=True)


def _to_col(row):
    return jnp.broadcast_to(row, (128, row.shape[1])).T


def _kernel(x_hbm, wqkv_hbm, wo_hbm, bx_hbm, wr_hbm, wg_hbm, wu_hbm, wd_hbm, gw_hbm,
            o_hbm,
            wr_v, gw_v, x_v, bx_v, wq_v, wk_v, wv_v, wo_v, wg_v, wu_v, wd_v,
            pqn_v, m_v, g_v, xcol_v, o_v,
            sems):
    copy = pltpu.make_async_copy

    def blk(i, n):
        return slice(i * n, (i + 1) * n)

    x_ = [(x_hbm.at[lo:hi], x_v.at[lo:hi]) for lo, hi in X_CHUNKS]
    kq_ = [[(wqkv_hbm.at[:, blk(NK + b, RK)], wk_v.at[b]), (wqkv_hbm.at[:, blk(b, RK)], wq_v.at[b])]
           for b in range(NK)]
    vo_ = [[(wqkv_hbm.at[:, blk(2 * NK + b, RK)], wv_v.at[b]),
            (wo_hbm.at[blk(b, RK)], wo_v.at[blk(b, RK)])] for b in range(NK)]
    ffn_ = [[(wg_hbm.at[:, lo:hi], wg_v.at[:, lo:hi]), (wu_hbm.at[:, lo:hi], wu_v.at[:, lo:hi]),
             (wd_hbm.at[lo:hi], wd_v.at[lo:hi])] for lo, hi in F_CHUNKS]
    groups = [kq_[0][:1], kq_[0][1:], x_[0:1], [(gw_hbm, gw_v), (wr_hbm, wr_v)], x_[1:2], x_[2:3],
              kq_[1] + x_[3:4], vo_[0] + [(bx_hbm, bx_v)] + kq_[2], ffn_[0], kq_[3] + vo_[1] + ffn_[1],
              vo_[2] + ffn_[2], vo_[3] + ffn_[3]]

    def start(i):
        for src, dst in groups[i]:
            copy(src, dst, sems.at[i]).start()

    def wait(i):
        for src, dst in groups[i]:
            copy(src, dst, sems.at[i]).wait()

    for i in range(4):
        start(i)
    wait(0)
    wk_t = wk_v[0].T
    start(4)
    wait(1)
    wq_t = wq_v[0].T
    wait(3)
    w_r = wr_v[...].astype(F32).reshape(1, D)
    g_w = gw_v[...].astype(F32).reshape(1, D)
    g_bits = pltpu.bitcast(jnp.broadcast_to(g_w[:, 0:128], (8, 128)), jnp.int32)
    always = (g_bits | 1) != 0
    same_head = (lax.broadcasted_iota(jnp.int32, (128, 128), 0) // DH
                 == lax.broadcasted_iota(jnp.int32, (128, 128), 1) // DH)

    st = {"best": jnp.full((16, 1), -jnp.inf, F32), "idx": jnp.zeros((16, 1), jnp.int32),
          "y": [jnp.zeros((8, 128), F32)] * (D // 128),
          "prev": [jnp.zeros((8, 128), F32)] * 2, "after": jnp.zeros((8, 128), F32)}

    def bits(v):
        return pltpu.bitcast(v, jnp.int32)

    def matmul(lhs, rhs, side, rhs_t=False, acc=None):
        m, k = lhs.shape
        site = 0
        for c in range(0, k, 512):
            first = [lhs[blk(i, 16), c:c + 128] for i in range(m // 16)]
            for i in range(0, m // 16, 8):
                prev = st["prev"][-(512 // m)]
                st["after"] = prev[blk(i * 16 * prev.shape[0] // m // 8, 8)]
                vals = [next(gen, None) for gen, stride in side if site % stride == 0]
                site += 1
                for v in vals:
                    if v is not None:
                        first[i] = pltpu.bitcast(jnp.where(always, bits(first[i]), bits(v)), BF16)
            a = jnp.concatenate([jnp.concatenate(first, axis=0), lhs[:, c + 128:c + 512]], axis=1)
            if rhs_t:
                part = lax.dot_general(a, rhs[:, c:c + 512], (((1,), (1,)), ((), ())),
                                       preferred_element_type=F32)
            else:
                part = jnp.dot(a, rhs[c:c + 512, :], preferred_element_type=F32)
            st["prev"].append(part)
            acc = part if acc is None else acc + part
        return acc

    def held(v):
        reps = (v.shape[0] // 8, v.shape[1] // 128)
        return jnp.where(jnp.tile(always, reps), v, jnp.tile(st["after"], reps))

    def transpose_work(name, w_v, b):
        cols = []
        for j in range(D // 128):
            cols.append(pltpu.bitcast(held(pltpu.bitcast(w_v[b, blk(j, 128), :], F32)), BF16).T)
            if j == D // 128 - 1:
                st[name] = jnp.concatenate(cols, axis=1)
            yield bits(cols[-1][112:128]) | bits(cols[-1][240:256])

    def norm_work(b, pq, z):
        zb = jnp.broadcast_to(z, (RK, 128))
        heads = range(RK // DH)
        for j in range(S // 128):
            ph = [pq[j][blk(h, DH)].astype(F32) for h in heads]
            den = [jnp.sum(ph[h] * zb[blk(h, DH)], axis=0, keepdims=True) for h in heads]
            inv = 1.0 / (held(jnp.concatenate(den, axis=0)) + 1e-6)
            yield inv
            inv = held(inv)
            out = jnp.concatenate([(ph[h] * inv[h:h + 1]).astype(BF16) for h in heads], axis=0).T
            pqn_v[blk(j, 128), blk(b, RK)] = out
            yield bits(out[112:128, 0:128]) | bits(out[112:128, 128:256])

    def route_work():
        g_w8, w_r8 = jnp.broadcast_to(g_w, (8, D)), jnp.broadcast_to(w_r, (8, D))
        for t in range(0, S, 16):
            g = _sigmoid(_rowdot(x_v[t:t + 16, :], g_w8, held))
            g_v[t:t + 16, :] = jnp.broadcast_to(g, (16, 128))
            r = _rbf(_rowdot(bx_v[t:t + 16, :], w_r8, held))
            better = r > st["best"]
            st["best"] = jnp.where(better, r, st["best"])
            st["idx"] = jnp.where(better, t, st["idx"])
            both = g + st["best"]
            yield jnp.broadcast_to(both[0:8] + both[8:16], (8, 128))

    def select_work():
        best = jnp.max(st["best"], axis=0, keepdims=True)
        pos = st["idx"] + lax.broadcasted_iota(jnp.int32, (16, 1), 0)
        idx = jnp.min(jnp.where(st["best"] == best, pos, S - 1), axis=0, keepdims=True)[0, 0]
        idx = jnp.clip(idx, 0, S - 1)
        grp = pl.multiple_of((idx // 16) * 16, 16)
        sel = lax.broadcasted_iota(jnp.int32, (16, 1), 0) == idx - grp
        b_grp = bx_v[pl.ds(grp, 16), :].astype(F32)
        xcol = _to_col(jnp.sum(jnp.where(sel, b_grp, 0.0), axis=0, keepdims=True))
        xcol_v[...] = xcol
        st.update(score=best, tok=idx)
        yield xcol[D - 8:D]

    def ffn_work(lo, hi):
        for c in range(lo, hi, 128):
            acc = []
            for w_v in (wg_v, wu_v):
                a = jnp.zeros((8, 128), F32)
                for k in range(D // 16):
                    if k in (0, 22, 43):
                        a = held(a)
                    pr = w_v[blk(k, 16), c:c + 128].astype(F32) * xcol_v[blk(k, 16), :]
                    a = a + pr[0:8] + pr[8:16]
                    if k in (21, 42, 63):
                        yield a
                acc.append(_rbf(jnp.sum(a, axis=0, keepdims=True)))
            gate, up = acc
            hcol = _to_col(_rbf(_rbf(gate * _sigmoid(gate)) * up))
            for n in range(D // 128):
                y = held(st["y"][n])
                for k in range(128 // 16):
                    pr = wd_v[c + k * 16:c + (k + 1) * 16, blk(n, 128)].astype(F32) * hcol[blk(k, 16)]
                    y = y + pr[0:8] + pr[8:16]
                st["y"][n] = y
                if n in (2, 5):
                    yield y + st["y"][n - 1] + st["y"][n - 2]
                if n == 7:
                    yield y + st["y"][n - 1]

    def after(sites, *gens):
        yield from [None] * sites
        for gen in gens:
            yield from gen

    def drain(gen):
        for _ in gen:
            pass

    def mix_work(b, gm):
        kv = []
        for i in range(RK // 128):
            t = jnp.dot(gm[blk(i, 128)], wv_v[b, :, blk(i, 128)], preferred_element_type=F32)
            kv.append(jnp.where(same_head, t, 0.0).astype(BF16))
        yield
        for i in range(RK // 128):
            rows = blk(b * (RK // 128) + i, 128)
            m_v[rows, :] = jnp.dot(kv[i], wo_v[rows, :], preferred_element_type=F32).astype(BF16)
        yield

    def k_step(b, mix, side, g_side, arrive=None):
        wt = jnp.concatenate([st["wk"], st["wq"]], axis=0)
        pk, pq, zacc = [], [], None
        for j in range(S // 128):
            if arrive is not None:
                arrive(j)
            p = _phi(matmul(wt, x_v[blk(j, 128), :], side, rhs_t=True)).astype(BF16)
            pk.append(p[0:RK])
            pq.append(p[RK:2 * RK])
            zacc = pk[j].astype(F32) if j == 0 else zacc + pk[j].astype(F32)
            next(mix, None)
        z = _rbf(jnp.sum(zacc, axis=1, keepdims=True))
        pk = jnp.concatenate(pk, axis=1)
        if arrive is not None:
            arrive(S // 128)
        own = [transpose_work(n, w, b + 1) for n, w in (("wk", wk_v), ("wq", wq_v)) if b + 1 < NK]
        norm = norm_work(b, pq, z)
        gm = [matmul(pk, x_v[:, blk(n, 128)],
                     [(norm, 2)] + [(w, 2) for w in own[n // 4:n // 4 + 1]] + g_side).astype(BF16)
              for n in range(D // 128)]
        for gen in own + [norm]:
            drain(gen)
        return mix_work(b, jnp.concatenate(gm, axis=1))

    def arrive(j):
        for i, (lo, _) in enumerate(X_CHUNKS):
            if lo == j * 128:
                start(5 + i)
                wait(3 + i if i else 2)

    st.update(wk=wk_t, wq=wq_t)
    mix = k_step(0, iter(()), [], [], arrive)

    start(9)
    wait(7)
    route = after(6, route_work(), after(8, select_work()))
    mix = k_step(1, mix, [(route, 1)], [(route, 1)])
    drain(route)

    start(10)
    wait(8)
    wait(9)
    ffn = after(6, ffn_work(F_CHUNKS[0][0], F_CHUNKS[1][1]))
    mix = k_step(2, mix, [(ffn, 1)], [])
    drain(ffn)

    def arrive_last(j):
        if j == S // 128:
            drain(ffn)
            wait(11)

    start(11)
    wait(10)
    ffn, ffn_last = after(6, ffn_work(*F_CHUNKS[2])), after(6, ffn_work(*F_CHUNKS[3]))
    mix = k_step(3, mix, [(ffn, 1)], [(ffn_last, 1)], arrive_last)
    drain(ffn_last)

    y = _rbf(jnp.sum(jnp.concatenate(st["y"], axis=1), axis=0, keepdims=True))
    y = _rbf(y * _rbf(_sigmoid(st["score"])))
    cp_o = []
    for t in range(NO):
        rows = blk(t, TO)
        g = g_v[rows, :]
        routed = lax.broadcasted_iota(jnp.int32, (TO, 128), 0) == st["tok"] - t * TO
        half = {}
        if t == 0:
            for n in range(4):
                half[n] = matmul(pqn_v[rows, 0:512], m_v[0:512, blk(n, 128)], [])
                next(mix, None)
        for n in range(D // 128):
            if n in half:
                a = matmul(pqn_v[rows, 512:D], m_v[512:D, blk(n, 128)], [], acc=half[n])
            else:
                a = matmul(pqn_v[rows, :], m_v[:, blk(n, 128)], [])
            bt = bx_v[rows, blk(n, 128)].astype(F32)
            bt = bt + (bt * 0.0 + jnp.where(routed, y[:, blk(n, 128)], 0.0))
            o_v[rows, blk(n, 128)] = (g * a + (1.0 - g) * bt).astype(BF16)
            if n + 1 in (O_STRIPS if t == NO - 1 else O_STRIPS[-1:]):
                lo = 0 if t < NO - 1 else ((0,) + O_STRIPS)[O_STRIPS.index(n + 1)]
                cols = slice(lo * 128, (n + 1) * 128)
                cp_o.append(copy(o_v.at[rows, cols], o_hbm.at[rows, cols], sems.at[len(groups) + len(cp_o)]))
                cp_o[-1].start()
    for c in cp_o:
        c.wait()


@jax.jit
def pallas_gated_mix__linear_attn_block__moe_arch_mod__prompt_kernel(
    A_x: jax.Array,
    A_wqkv: jax.Array,
    A_wo: jax.Array,
    B_x: jax.Array,
    B_w_r: jax.Array,
    B_w_gate: jax.Array,
    B_w_up: jax.Array,
    B_w_down: jax.Array,
    gate_w: jax.Array,
):
    hbm = pl.BlockSpec(memory_space=pl.ANY)
    out = pl.pallas_call(
        _kernel,
        out_shape=jax.ShapeDtypeStruct((S, D), BF16),
        in_specs=[hbm] * 9,
        out_specs=hbm,
        scratch_shapes=[
            pltpu.VMEM((D,), BF16),
            pltpu.VMEM((D,), BF16),
            pltpu.VMEM((S, D), BF16),
            pltpu.VMEM((S, D), BF16),
            pltpu.VMEM((NK, D, RK), BF16),
            pltpu.VMEM((NK, D, RK), BF16),
            pltpu.VMEM((NK, D, RK), BF16),
            pltpu.VMEM((D, D), BF16),
            pltpu.VMEM((D, F), BF16),
            pltpu.VMEM((D, F), BF16),
            pltpu.VMEM((F, D), BF16),
            pltpu.VMEM((S, D), BF16),
            pltpu.VMEM((D, D), BF16),
            pltpu.VMEM((S, 128), F32),
            pltpu.VMEM((D, 128), F32),
            pltpu.VMEM((S, D), BF16),
            pltpu.SemaphoreType.DMA((N_GROUPS + NO - 1 + len(O_STRIPS),)),
        ],
        compiler_params=pltpu.CompilerParams(vmem_limit_bytes=100 * 1024 * 1024),
    )(A_x.reshape(S, D), A_wqkv, A_wo, B_x.reshape(S, D), B_w_r,
      B_w_gate, B_w_up, B_w_down, gate_w)
    return out.reshape(1, S, D)
```

```python
import jax
import jax.numpy as jnp
from jax import lax
import jax.experimental.pallas as pl
import jax.experimental.pallas.tpu as pltpu

S, D, F, H = 2048, 1024, 3584, 32
DH = D // H
RK = 256
TO = 512
NK, NO = D // RK, S // TO
F_CHUNKS = ((0, 768), (768, 1536), (1536, 2944), (2944, 3584))
NF = len(F_CHUNKS)
X_CHUNKS = ((0, 256), (256, 640), (640, 1280), (1280, 2048))
O_STRIPS = (3, 5, 7, 8)
N_GROUPS = 12
F32, BF16 = jnp.float32, jnp.bfloat16


def _phi(t):
    return jnp.where(t > 0, t + 1.0, jnp.exp(t)) + 1e-6


def _sigmoid(t):
    return 1.0 / (1.0 + jnp.exp(-t))


def _rbf(t):
    return t.astype(BF16).astype(F32)


def _rowdot(a, w, first):
    acc = None
    for j in range(0, D, 128):
        wj = first(w[:, 0:128]) if j == 0 else w[:, j:j + 128]
        pr = a[:, j:j + 128].astype(F32) * jnp.concatenate([wj, wj], axis=0)
        acc = pr if j == 0 else acc + pr
    return jnp.sum(acc, axis=1, keepdims=True)


def _to_col(row):
    return jnp.broadcast_to(row, (128, row.shape[1])).T


def _kernel(x_hbm, wqkv_hbm, wo_hbm, bx_hbm, wr_hbm, wg_hbm, wu_hbm, wd_hbm, gw_hbm,
            o_hbm,
            wr_v, gw_v, x_v, bx_v, wq_v, wk_v, wv_v, wo_v, wg_v, wu_v, wd_v,
            pqn_v, m_v, g_v, xcol_v, o_v,
            sems):
    copy = pltpu.make_async_copy

    def blk(i, n):
        return slice(i * n, (i + 1) * n)

    x_ = [(x_hbm.at[lo:hi], x_v.at[lo:hi]) for lo, hi in X_CHUNKS]
    kq_ = [[(wqkv_hbm.at[:, blk(NK + b, RK)], wk_v.at[b]), (wqkv_hbm.at[:, blk(b, RK)], wq_v.at[b])]
           for b in range(NK)]
    vo_ = [[(wqkv_hbm.at[:, blk(2 * NK + b, RK)], wv_v.at[b]),
            (wo_hbm.at[blk(b, RK)], wo_v.at[blk(b, RK)])] for b in range(NK)]
    ffn_ = [[(wg_hbm.at[:, lo:hi], wg_v.at[:, lo:hi]), (wu_hbm.at[:, lo:hi], wu_v.at[:, lo:hi]),
             (wd_hbm.at[lo:hi], wd_v.at[lo:hi])] for lo, hi in F_CHUNKS]
    groups = [kq_[0][:1], kq_[0][1:], x_[0:1], [(gw_hbm, gw_v), (wr_hbm, wr_v)], x_[1:2], x_[2:3],
              kq_[1] + x_[3:4], vo_[0] + [(bx_hbm, bx_v)] + kq_[2], ffn_[0], kq_[3] + vo_[1] + ffn_[1],
              vo_[2] + ffn_[2], vo_[3] + ffn_[3]]

    def start(i):
        for src, dst in groups[i]:
            copy(src, dst, sems.at[i]).start()

    def wait(i):
        for src, dst in groups[i]:
            copy(src, dst, sems.at[i]).wait()

    for i in range(4):
        start(i)
    wait(0)
    wk_t = wk_v[0].T
    start(4)
    wait(1)
    wq_t = wq_v[0].T
    wait(3)
    w_r = wr_v[...].astype(F32).reshape(1, D)
    g_w = gw_v[...].astype(F32).reshape(1, D)
    g_bits = pltpu.bitcast(jnp.broadcast_to(g_w[:, 0:128], (8, 128)), jnp.int32)
    always = (g_bits | 1) != 0
    same_head = (lax.broadcasted_iota(jnp.int32, (128, 128), 0) // DH
                 == lax.broadcasted_iota(jnp.int32, (128, 128), 1) // DH)

    st = {"best": jnp.full((16, 1), -jnp.inf, F32), "idx": jnp.zeros((16, 1), jnp.int32),
          "y": [jnp.zeros((8, 128), F32)] * (D // 128),
          "prev": [jnp.zeros((8, 128), F32)] * 2, "after": jnp.zeros((8, 128), F32)}

    def bits(v):
        return pltpu.bitcast(v, jnp.int32)

    def matmul(lhs, rhs, side, rhs_t=False, acc=None):
        m, k = lhs.shape
        for c in range(0, k, 512):
            first = [lhs[blk(i, 16), c:c + 128] for i in range(m // 16)]
            for i in range(0, m // 16, 8):
                prev = st["prev"][-(512 // m)]
                st["after"] = prev[blk(i * 16 * prev.shape[0] // m // 8, 8)]
                for v in [v for gen in side for v in next(gen, ())]:
                    first[i] = pltpu.bitcast(jnp.where(always, bits(first[i]), bits(v)), BF16)
            a = jnp.concatenate([jnp.concatenate(first, axis=0), lhs[:, c + 128:c + 512]], axis=1)
            if rhs_t:
                part = lax.dot_general(a, rhs[:, c:c + 512], (((1,), (1,)), ((), ())),
                                       preferred_element_type=F32)
            else:
                part = jnp.dot(a, rhs[c:c + 512, :], preferred_element_type=F32)
            st["prev"].append(part)
            acc = part if acc is None else acc + part
        return acc

    def held(v):
        reps = (v.shape[0] // 8, v.shape[1] // 128)
        return jnp.where(jnp.tile(always, reps), v, jnp.tile(st["after"], reps))

    def transpose_work(name, w_v, b):
        cols = []
        for j in range(D // 128):
            cols.append(pltpu.bitcast(held(pltpu.bitcast(w_v[b, blk(j, 128), :], F32)), BF16).T)
            if j == D // 128 - 1:
                st[name] = jnp.concatenate(cols, axis=1)
            yield bits(cols[-1][112:128]) | bits(cols[-1][240:256])

    def norm_work(b, pq, z):
        zb = jnp.broadcast_to(z, (RK, 128))
        heads = range(RK // DH)
        for j in range(S // 128):
            ph = [pq[j][blk(h, DH)].astype(F32) for h in heads]
            den = [jnp.sum(ph[h] * zb[blk(h, DH)], axis=0, keepdims=True) for h in heads]
            inv = 1.0 / (held(jnp.concatenate(den, axis=0)) + 1e-6)
            yield inv
            inv = held(inv)
            out = jnp.concatenate([(ph[h] * inv[h:h + 1]).astype(BF16) for h in heads], axis=0).T
            pqn_v[blk(j, 128), blk(b, RK)] = out
            yield bits(out[112:128, 0:128]) | bits(out[112:128, 128:256])

    def route_work():
        g_w8, w_r8 = jnp.broadcast_to(g_w, (8, D)), jnp.broadcast_to(w_r, (8, D))
        for t in range(0, S, 16):
            g = _sigmoid(_rowdot(x_v[t:t + 16, :], g_w8, held))
            g_v[t:t + 16, :] = jnp.broadcast_to(g, (16, 128))
            r = _rbf(_rowdot(bx_v[t:t + 16, :], w_r8, held))
            better = r > st["best"]
            st["best"] = jnp.where(better, r, st["best"])
            st["idx"] = jnp.where(better, t, st["idx"])
            both = g + st["best"]
            yield jnp.broadcast_to(both[0:8] + both[8:16], (8, 128))

    def select_work():
        best = jnp.max(st["best"], axis=0, keepdims=True)
        pos = st["idx"] + lax.broadcasted_iota(jnp.int32, (16, 1), 0)
        idx = jnp.min(jnp.where(st["best"] == best, pos, S - 1), axis=0, keepdims=True)[0, 0]
        idx = jnp.clip(idx, 0, S - 1)
        grp = pl.multiple_of((idx // 16) * 16, 16)
        sel = lax.broadcasted_iota(jnp.int32, (16, 1), 0) == idx - grp
        b_grp = bx_v[pl.ds(grp, 16), :].astype(F32)
        xcol = _to_col(jnp.sum(jnp.where(sel, b_grp, 0.0), axis=0, keepdims=True))
        xcol_v[...] = xcol
        st.update(score=best, tok=idx)
        yield xcol[D - 8:D]

    def ffn_work(lo, hi):
        for c in range(lo, hi, 128):
            acc = []
            for w_v in (wg_v, wu_v):
                a = jnp.zeros((8, 128), F32)
                for k in range(D // 16):
                    if k in (0, 22, 43):
                        a = held(a)
                    pr = w_v[blk(k, 16), c:c + 128].astype(F32) * xcol_v[blk(k, 16), :]
                    a = a + pr[0:8] + pr[8:16]
                    if k in (21, 42, 63):
                        yield a
                acc.append(_rbf(jnp.sum(a, axis=0, keepdims=True)))
            gate, up = acc
            hcol = _to_col(_rbf(_rbf(gate * _sigmoid(gate)) * up))
            for n in range(D // 128):
                y = held(st["y"][n])
                for k in range(128 // 16):
                    pr = wd_v[c + k * 16:c + (k + 1) * 16, blk(n, 128)].astype(F32) * hcol[blk(k, 16)]
                    y = y + pr[0:8] + pr[8:16]
                st["y"][n] = y
                if n in (2, 5):
                    yield y + st["y"][n - 1] + st["y"][n - 2]
                if n == 7:
                    yield y + st["y"][n - 1]

    def paced(gen, n, lo, hi):
        for site in range(hi):
            due = max(site + 1 - lo, 0) * n // (hi - lo) - max(site - lo, 0) * n // (hi - lo)
            yield [next(gen) for _ in range(due)]
        assert next(gen, None) is None

    def finish(side):
        for gen in side:
            assert next(gen, None) is None

    def mix_work(b, gm):
        kv = []
        for i in range(RK // 128):
            t = jnp.dot(gm[blk(i, 128)], wv_v[b, :, blk(i, 128)], preferred_element_type=F32)
            kv.append(jnp.where(same_head, t, 0.0).astype(BF16))
        yield
        for i in range(RK // 128):
            rows = blk(b * (RK // 128) + i, 128)
            m_v[rows, :] = jnp.dot(kv[i], wo_v[rows, :], preferred_element_type=F32).astype(BF16)
        yield

    def k_step(b, mix, arrive, kq_side=(), g_side=()):
        wt = jnp.concatenate([st["wk"], st["wq"]], axis=0)
        pk, pq, zacc = [], [], None
        for j in range(S // 128):
            arrive(j)
            p = _phi(matmul(wt, x_v[blk(j, 128), :], kq_side, rhs_t=True)).astype(BF16)
            pk.append(p[0:RK])
            pq.append(p[RK:2 * RK])
            zacc = pk[j].astype(F32) if j == 0 else zacc + pk[j].astype(F32)
            if j in (0, 2):
                next(mix, None)
        finish(kq_side)
        z = _rbf(jnp.sum(zacc, axis=1, keepdims=True))
        pk = jnp.concatenate(pk, axis=1)
        side = [paced(norm_work(b, pq, z), 2 * S // 128, 4, 57), *g_side]
        if b + 1 < NK:
            side += [paced(transpose_work("wk", wk_v, b + 1), D // 128, 0, 28),
                     paced(transpose_work("wq", wq_v, b + 1), D // 128, 28, 56)]
        gm = []
        for n in range(D // 128):
            arrive(S // 128 + n)
            gm.append(matmul(pk, x_v[:, blk(n, 128)], side).astype(BF16))
        finish(side)
        return mix_work(b, jnp.concatenate(gm, axis=1))

    def arrivals(plan):
        def arrive(j):
            starts, waits = plan.get(j, ((), ()))
            for i in starts:
                start(i)
            for i in waits:
                wait(i)
        return arrive

    def ffn(lo, hi, first, last):
        return [paced(ffn_work(lo, hi), (hi - lo) // 128 * 9, first, last)]

    st.update(wk=wk_t, wq=wq_t)
    mix = k_step(0, iter(()), arrivals(
        {lo // 128: ((5 + i,), (3 + i if i else 2,)) for i, (lo, _) in enumerate(X_CHUNKS)}))
    mix = k_step(1, mix, arrivals({0: ((9,), (7,))}),
                 [paced(route_work(), S // 16, 6, 128)], [paced(select_work(), 1, 12, 13)])
    mix = k_step(2, mix, arrivals({0: ((10,), (8, 9))}),
                 ffn(F_CHUNKS[0][0], F_CHUNKS[1][1], 6, 126))
    mix = k_step(3, mix, arrivals({0: ((11,), (10,)), S // 128: ((), (11,))}),
                 ffn(*F_CHUNKS[2], 6, 126), ffn(*F_CHUNKS[3], 6, 58))

    y = _rbf(jnp.sum(jnp.concatenate(st["y"], axis=1), axis=0, keepdims=True))
    y = _rbf(y * _rbf(_sigmoid(st["score"])))
    cp_o = []
    for t in range(NO):
        rows = blk(t, TO)
        g = g_v[rows, :]
        routed = lax.broadcasted_iota(jnp.int32, (TO, 128), 0) == st["tok"] - t * TO
        half = {}
        if t == 0:
            for n in range(4):
                half[n] = matmul(pqn_v[rows, 0:512], m_v[0:512, blk(n, 128)], [])
                next(mix, None)
        for n in range(D // 128):
            if n in half:
                a = matmul(pqn_v[rows, 512:D], m_v[512:D, blk(n, 128)], [], acc=half[n])
            else:
                a = matmul(pqn_v[rows, :], m_v[:, blk(n, 128)], [])
            bt = bx_v[rows, blk(n, 128)].astype(F32)
            bt = bt + (bt * 0.0 + jnp.where(routed, y[:, blk(n, 128)], 0.0))
            o_v[rows, blk(n, 128)] = (g * a + (1.0 - g) * bt).astype(BF16)
            if n + 1 in (O_STRIPS if t == NO - 1 else O_STRIPS[-1:]):
                lo = 0 if t < NO - 1 else ((0,) + O_STRIPS)[O_STRIPS.index(n + 1)]
                cols = slice(lo * 128, (n + 1) * 128)
                cp_o.append(copy(o_v.at[rows, cols], o_hbm.at[rows, cols], sems.at[len(groups) + len(cp_o)]))
                cp_o[-1].start()
    for c in cp_o:
        c.wait()


@jax.jit
def pallas_gated_mix__linear_attn_block__moe_arch_mod__prompt_kernel(
    A_x: jax.Array,
    A_wqkv: jax.Array,
    A_wo: jax.Array,
    B_x: jax.Array,
    B_w_r: jax.Array,
    B_w_gate: jax.Array,
    B_w_up: jax.Array,
    B_w_down: jax.Array,
    gate_w: jax.Array,
):
    hbm = pl.BlockSpec(memory_space=pl.ANY)
    out = pl.pallas_call(
        _kernel,
        out_shape=jax.ShapeDtypeStruct((S, D), BF16),
        in_specs=[hbm] * 9,
        out_specs=hbm,
        scratch_shapes=[
            pltpu.VMEM((D,), BF16),
            pltpu.VMEM((D,), BF16),
            pltpu.VMEM((S, D), BF16),
            pltpu.VMEM((S, D), BF16),
            pltpu.VMEM((NK, D, RK), BF16),
            pltpu.VMEM((NK, D, RK), BF16),
            pltpu.VMEM((NK, D, RK), BF16),
            pltpu.VMEM((D, D), BF16),
            pltpu.VMEM((D, F), BF16),
            pltpu.VMEM((D, F), BF16),
            pltpu.VMEM((F, D), BF16),
            pltpu.VMEM((S, D), BF16),
            pltpu.VMEM((D, D), BF16),
            pltpu.VMEM((S, 128), F32),
            pltpu.VMEM((D, 128), F32),
            pltpu.VMEM((S, D), BF16),
            pltpu.SemaphoreType.DMA((N_GROUPS + NO - 1 + len(O_STRIPS),)),
        ],
        compiler_params=pltpu.CompilerParams(vmem_limit_bytes=100 * 1024 * 1024),
    )(A_x.reshape(S, D), A_wqkv, A_wo, B_x.reshape(S, D), B_w_r,
      B_w_gate, B_w_up, B_w_down, gate_w)
    return out.reshape(1, S, D)
```

```python
import jax
import jax.numpy as jnp
from jax import lax
import jax.experimental.pallas as pl
import jax.experimental.pallas.tpu as pltpu

S, D, F, H = 2048, 1024, 3584, 32
DH = D // H
RK = 256
TO = 512
NK, NO = D // RK, S // TO
F_CHUNKS = ((0, 896), (896, 1792), (1792, 3584))
X_CHUNKS = ((0, 384), (384, 768), (768, 1408), (1408, 2048))
O_STRIPS = (3, 5, 7, 8)
N_GROUPS = 10
F32, BF16 = jnp.float32, jnp.bfloat16


def _phi(t):
    return jnp.where(t > 0, t + 1.0, jnp.exp(t)) + 1e-6


def _sigmoid(t):
    return 1.0 / (1.0 + jnp.exp(-t))


def _rbf(t):
    return t.astype(BF16).astype(F32)


def _rowdot(a, w, first):
    acc = None
    for j in range(0, D, 128):
        wj = first(w[:, 0:128]) if j == 0 else w[:, j:j + 128]
        pr = a[:, j:j + 128] * jnp.concatenate([wj, wj], axis=0)
        acc = pr if j == 0 else acc + pr
    return jnp.sum(acc, axis=1, keepdims=True)


def _to_col(row):
    return jnp.broadcast_to(row, (128, row.shape[1])).T


def _kernel(x_hbm, wqkv_hbm, wo_hbm, wr_hbm, wg_hbm, wu_hbm, wd_hbm, gw_hbm,
            o_hbm,
            wr_v, gw_v, x_v, wq_v, wk_v, wv_v, wo_v, wg_v, wu_v, wd_v,
            pqn_v, m_v, g_v, xcol_v, o_v,
            sems):
    copy = pltpu.make_async_copy

    def blk(i, n):
        return slice(i * n, (i + 1) * n)

    x_ = [(x_hbm.at[lo:hi], x_v.at[lo:hi]) for lo, hi in X_CHUNKS]
    kq_ = [[(wqkv_hbm.at[:, blk(NK + b, RK)], wk_v.at[b]), (wqkv_hbm.at[:, blk(b, RK)], wq_v.at[b])]
           for b in range(NK)]
    vo_ = [[(wqkv_hbm.at[:, blk(2 * NK + b, RK)], wv_v.at[b]),
            (wo_hbm.at[blk(b, RK)], wo_v.at[blk(b, RK)])] for b in range(NK)]
    ffn_ = [[(wg_hbm.at[:, lo:hi], wg_v.at[:, lo:hi]), (wu_hbm.at[:, lo:hi], wu_v.at[:, lo:hi]),
             (wd_hbm.at[lo:hi], wd_v.at[lo:hi])] for lo, hi in F_CHUNKS]
    groups = [kq_[0][:1], x_[0:1] + [(gw_hbm, gw_v), (wr_hbm, wr_v)], kq_[0][1:], x_[1:2], x_[2:3],
              kq_[1] + x_[3:4], vo_[0] + kq_[2], ffn_[0], kq_[3] + vo_[1] + ffn_[1],
              vo_[2] + vo_[3] + ffn_[2]]

    def start(i):
        for src, dst in groups[i]:
            copy(src, dst, sems.at[i]).start()

    def wait(i):
        for src, dst in groups[i]:
            copy(src, dst, sems.at[i]).wait()

    for i in range(3):
        start(i)
    wait(0)
    wk_t = wk_v[0].T
    start(3)
    wait(1)
    w_r = wr_v[...].astype(F32).reshape(1, D)
    g_w = gw_v[...].astype(F32).reshape(1, D)
    g_bits = pltpu.bitcast(jnp.broadcast_to(g_w[:, 0:128], (8, 128)), jnp.int32)
    always = (g_bits | 1) != 0
    same_head = (lax.broadcasted_iota(jnp.int32, (128, 128), 0) // DH
                 == lax.broadcasted_iota(jnp.int32, (128, 128), 1) // DH)

    st = {"best": jnp.full((16, 1), -jnp.inf, F32), "idx": jnp.zeros((16, 1), jnp.int32),
          "y": [jnp.zeros((8, 128), F32)] * (D // 128),
          "prev": [jnp.zeros((8, 128), F32)] * 2, "after": jnp.zeros((8, 128), F32)}

    def bits(v):
        return pltpu.bitcast(v, jnp.int32)

    def matmul(lhs, rhs, side, rhs_t=False, acc=None):
        m, k = lhs.shape
        for c in range(0, k, 512):
            first = [lhs[blk(i, 16), c:c + 128] for i in range(m // 16)]
            for i in range(0, m // 16, 8):
                prev = st["prev"][-(512 // m)]
                st["after"] = prev[blk(i * 16 * prev.shape[0] // m // 8, 8)]
                for v in [v for gen in side for v in next(gen, ())]:
                    first[i] = pltpu.bitcast(jnp.where(always, bits(first[i]), bits(v)), BF16)
            a = jnp.concatenate([jnp.concatenate(first, axis=0), lhs[:, c + 128:c + 512]], axis=1)
            if rhs_t:
                part = lax.dot_general(a, rhs[:, c:c + 512], (((1,), (1,)), ((), ())),
                                       preferred_element_type=F32)
            else:
                part = jnp.dot(a, rhs[c:c + 512, :], preferred_element_type=F32)
            st["prev"].append(part)
            acc = part if acc is None else acc + part
        return acc

    def held(v):
        reps = (v.shape[0] // 8, v.shape[1] // 128)
        return jnp.where(jnp.tile(always, reps), v, jnp.tile(st["after"], reps))

    def transpose_work(name, w_v, b):
        cols = []
        for j in range(D // 128):
            cols.append(pltpu.bitcast(held(pltpu.bitcast(w_v[b, blk(j, 128), :], F32)), BF16).T)
            if j == D // 128 - 1:
                st[name] = jnp.concatenate(cols, axis=1)
            yield bits(cols[-1][112:128]) | bits(cols[-1][240:256])

    def norm_work(b, pq, z):
        zb = jnp.broadcast_to(z, (RK, 128))
        heads = range(RK // DH)
        for j in range(S // 128):
            ph = [pq[j][blk(h, DH)].astype(F32) for h in heads]
            den = [jnp.sum(ph[h] * zb[blk(h, DH)], axis=0, keepdims=True) for h in heads]
            inv = 1.0 / (held(jnp.concatenate(den, axis=0)) + 1e-6)
            yield inv
            inv = held(inv)
            out = jnp.concatenate([(ph[h] * inv[h:h + 1]).astype(BF16) for h in heads], axis=0).T
            pqn_v[blk(j, 128), blk(b, RK)] = out
            yield bits(out[112:128, 0:128]) | bits(out[112:128, 128:256])

    def route_work():
        g_w8, w_r8 = jnp.broadcast_to(g_w, (8, D)), jnp.broadcast_to(w_r, (8, D))
        for t in range(0, S, 16):
            xt = x_v[t:t + 16, :].astype(F32)
            g = _sigmoid(_rowdot(xt, g_w8, held))
            g_v[t:t + 16, :] = jnp.broadcast_to(g, (16, 128))
            r = _rbf(_rowdot(xt, w_r8, held))
            better = r > st["best"]
            st["best"] = jnp.where(better, r, st["best"])
            st["idx"] = jnp.where(better, t, st["idx"])
            both = g + st["best"]
            yield jnp.broadcast_to(both[0:8] + both[8:16], (8, 128))

    def select_work():
        best = jnp.max(st["best"], axis=0, keepdims=True)
        pos = st["idx"] + lax.broadcasted_iota(jnp.int32, (16, 1), 0)
        idx = jnp.min(jnp.where(st["best"] == best, pos, S - 1), axis=0, keepdims=True)[0, 0]
        idx = jnp.clip(idx, 0, S - 1)
        grp = pl.multiple_of((idx // 16) * 16, 16)
        sel = lax.broadcasted_iota(jnp.int32, (16, 1), 0) == idx - grp
        rows = x_v[pl.ds(grp, 16), :].astype(F32)
        xcol = _to_col(jnp.sum(jnp.where(sel, rows, 0.0), axis=0, keepdims=True))
        xcol_v[...] = xcol
        st.update(score=best, tok=idx)
        yield xcol[D - 8:D]

    def ffn_work(lo, hi):
        for c in range(lo, hi, 128):
            acc = []
            for w_v in (wg_v, wu_v):
                a = jnp.zeros((8, 128), F32)
                for k in range(D // 16):
                    if k in (0, 22, 43):
                        a = held(a)
                    pr = w_v[blk(k, 16), c:c + 128].astype(F32) * xcol_v[blk(k, 16), :]
                    a = a + pr[0:8] + pr[8:16]
                    if k in (21, 42, 63):
                        yield a
                acc.append(_rbf(jnp.sum(a, axis=0, keepdims=True)))
            gate, up = acc
            hcol = _to_col(_rbf(_rbf(gate * _sigmoid(gate)) * up))
            for n in range(D // 128):
                y = held(st["y"][n])
                for k in range(128 // 16):
                    pr = wd_v[c + k * 16:c + (k + 1) * 16, blk(n, 128)].astype(F32) * hcol[blk(k, 16)]
                    y = y + pr[0:8] + pr[8:16]
                st["y"][n] = y
                if n in (2, 5):
                    yield y + st["y"][n - 1] + st["y"][n - 2]
                if n == 7:
                    yield y + st["y"][n - 1]

    def paced(gen, n, lo, hi):
        for site in range(hi):
            due = max(site + 1 - lo, 0) * n // (hi - lo) - max(site - lo, 0) * n // (hi - lo)
            yield [next(gen) for _ in range(due)]
        assert next(gen, None) is None

    def finish(side):
        for gen in side:
            assert next(gen, None) is None

    def mix_work(b, gm):
        kv = []
        for i in range(RK // 128):
            t = jnp.dot(gm[blk(i, 128)], wv_v[b, :, blk(i, 128)], preferred_element_type=F32)
            kv.append(jnp.where(same_head, t, 0.0).astype(BF16))
        yield
        for i in range(RK // 128):
            rows = blk(b * (RK // 128) + i, 128)
            m_v[rows, :] = jnp.dot(kv[i], wo_v[rows, :], preferred_element_type=F32).astype(BF16)
        yield

    def k_step(b, mix, arrive, kq_side=(), g_side=()):
        def proj(w_t, j):
            return _phi(matmul(w_t, x_v[blk(j, 128), :], kq_side, rhs_t=True)).astype(BF16)

        pk, pq = [], []
        if b == 0:
            pk = [proj(st["wk"], j) for j in range(X_CHUNKS[0][1] // 128)]
            wait(2)
            st["wq"] = wq_v[0].T
            pq = [proj(st["wq"], j) for j in range(len(pk))]
        wt = jnp.concatenate([st["wk"], st["wq"]], axis=0)
        for j in range(len(pk), S // 128):
            arrive(j)
            p = proj(wt, j)
            pk.append(p[0:RK])
            pq.append(p[RK:2 * RK])
            if j in (0, 2):
                next(mix, None)
        finish(kq_side)
        zacc = pk[0].astype(F32)
        for t in pk[1:]:
            zacc = zacc + t.astype(F32)
        z = _rbf(jnp.sum(zacc, axis=1, keepdims=True))
        pk = jnp.concatenate(pk, axis=1)
        side = [paced(norm_work(b, pq, z), 2 * S // 128, 4, 57), *g_side]
        if b + 1 < NK:
            side += [paced(transpose_work("wk", wk_v, b + 1), D // 128, 0, 28),
                     paced(transpose_work("wq", wq_v, b + 1), D // 128, 28, 56)]
        gm = []
        for n in range(D // 128):
            arrive(S // 128 + n)
            gm.append(matmul(pk, x_v[:, blk(n, 128)], side).astype(BF16))
        finish(side)
        return mix_work(b, jnp.concatenate(gm, axis=1))

    def arrivals(plan):
        def arrive(j):
            starts, waits = plan.get(j, ((), ()))
            for i in starts:
                start(i)
            for i in waits:
                wait(i)
        return arrive

    def ffn(lo, hi, first, last):
        return [paced(ffn_work(lo, hi), (hi - lo) // 128 * 9, first, last)]

    st["wk"] = wk_t
    mix = k_step(0, iter(()), arrivals(
        {lo // 128: ((3 + i,), (2 + i,)) for i, (lo, _) in enumerate(X_CHUNKS) if i} | {S // 128: ((7,), ())}))
    mix = k_step(1, mix, arrivals({0: ((8,), (6,))}),
                 [paced(route_work(), S // 16, 4, 120)], [paced(select_work(), 1, 12, 13)])
    mix = k_step(2, mix, arrivals({0: ((9,), (7, 8))}),
                 ffn(F_CHUNKS[0][0], F_CHUNKS[1][1], 4, 120))
    mix = k_step(3, mix, arrivals({0: ((), (9,))}), ffn(*F_CHUNKS[2], 4, 120))

    y = _rbf(jnp.sum(jnp.concatenate(st["y"], axis=1), axis=0, keepdims=True))
    y = _rbf(y * _rbf(_sigmoid(st["score"])))
    cp_o = []
    for t in range(NO):
        rows = blk(t, TO)
        g = g_v[rows, :]
        routed = lax.broadcasted_iota(jnp.int32, (TO, 128), 0) == st["tok"] - t * TO
        half = {}
        if t == 0:
            for n in range(4):
                half[n] = matmul(pqn_v[rows, 0:512], m_v[0:512, blk(n, 128)], [])
                next(mix, None)
        for n in range(D // 128):
            if n in half:
                a = matmul(pqn_v[rows, 512:D], m_v[512:D, blk(n, 128)], [], acc=half[n])
            else:
                a = matmul(pqn_v[rows, :], m_v[:, blk(n, 128)], [])
            bt = x_v[rows, blk(n, 128)].astype(F32)
            bt = bt + (bt * 0.0 + jnp.where(routed, y[:, blk(n, 128)], 0.0))
            o_v[rows, blk(n, 128)] = (g * a + (1.0 - g) * bt).astype(BF16)
            if n + 1 in (O_STRIPS if t == NO - 1 else O_STRIPS[-1:]):
                lo = 0 if t < NO - 1 else ((0,) + O_STRIPS)[O_STRIPS.index(n + 1)]
                cols = slice(lo * 128, (n + 1) * 128)
                cp_o.append(copy(o_v.at[rows, cols], o_hbm.at[rows, cols], sems.at[len(groups) + len(cp_o)]))
                cp_o[-1].start()
    for c in cp_o:
        c.wait()


@jax.jit
def pallas_gated_mix__linear_attn_block__moe_arch_mod__prompt_kernel(
    A_x: jax.Array,
    A_wqkv: jax.Array,
    A_wo: jax.Array,
    B_x: jax.Array,
    B_w_r: jax.Array,
    B_w_gate: jax.Array,
    B_w_up: jax.Array,
    B_w_down: jax.Array,
    gate_w: jax.Array,
):
    del B_x
    hbm = pl.BlockSpec(memory_space=pl.ANY)
    out = pl.pallas_call(
        _kernel,
        out_shape=jax.ShapeDtypeStruct((S, D), BF16),
        in_specs=[hbm] * 8,
        out_specs=hbm,
        scratch_shapes=[
            pltpu.VMEM((D,), BF16),
            pltpu.VMEM((D,), BF16),
            pltpu.VMEM((S, D), BF16),
            pltpu.VMEM((NK, D, RK), BF16),
            pltpu.VMEM((NK, D, RK), BF16),
            pltpu.VMEM((NK, D, RK), BF16),
            pltpu.VMEM((D, D), BF16),
            pltpu.VMEM((D, F), BF16),
            pltpu.VMEM((D, F), BF16),
            pltpu.VMEM((F, D), BF16),
            pltpu.VMEM((S, D), BF16),
            pltpu.VMEM((D, D), BF16),
            pltpu.VMEM((S, 128), F32),
            pltpu.VMEM((D, 128), F32),
            pltpu.VMEM((S, D), BF16),
            pltpu.SemaphoreType.DMA((N_GROUPS + NO - 1 + len(O_STRIPS),)),
        ],
        compiler_params=pltpu.CompilerParams(vmem_limit_bytes=100 * 1024 * 1024),
    )(A_x.reshape(S, D), A_wqkv, A_wo, B_w_r,
      B_w_gate, B_w_up, B_w_down, gate_w)
    return out.reshape(1, S, D)
```
